```python
import os as _os
_os.environ.setdefault('JAX_PLATFORMS', 'cpu')
import jax
import jax.numpy as jnp

def _softmax(x, axis=-1):
    return jax.nn.softmax(x, axis=axis)

def _gelu(x):
    return jax.nn.gelu(x, approximate=True)

def _silu(x):
    return jax.nn.silu(x)

def _sigmoid(x):
    return jax.nn.sigmoid(x)

def _layernorm(x, axis=-1, eps=1e-05):
    m = jnp.mean(x, axis=axis, keepdims=True)
    v = jnp.var(x, axis=axis, keepdims=True)
    return (x - m) / jnp.sqrt(v + eps)

def _scatter_add(tgt, idx, src, axis=0):
    return tgt.at[idx].add(src)

def _segment_sum(src, seg, n):
    return jax.ops.segment_sum(src, seg, n)

class _Rng:

    def __init__(self, key):
        self._k = key

    def _next(self):
        self._k, sub = jax.random.split(self._k)
        return sub

    def normal(self, shape):
        return jax.random.normal(self._next(), shape, dtype=jnp.bfloat16)

    def randint(self, lo, hi, shape):
        return jax.random.randint(self._next(), shape, lo, hi, dtype=jnp.int32)

    def uniform(self, shape, lo=0.0, hi=1.0):
        return jax.random.uniform(self._next(), shape, jnp.bfloat16, lo, hi)

    def permutation(self, n):
        return jax.random.permutation(self._next(), n)
kernel_name = 'adaLN_cond__grouped_kv_mqa__swiglu_ffn__prompt'

def setup_inputs():
    _rng = _Rng(jax.random.key(int.from_bytes(__import__("os").urandom(4), "little")))
    _w = lambda a: (lambda t: t.astype(jnp.bfloat16) if jnp.issubdtype(t.dtype, jnp.floating) else t)(jnp.asarray(a))

    def _A_setup():
        B, S, D, H = (1, 2048, 576, 32)
        Dh = D // H
        return {'x': _w((lambda *s: _rng.normal(s) * 0.05)(B, S, D)), 'wq': _w((lambda *s: _rng.normal(s) * 0.05)(D, H * Dh)), 'wk': _w((lambda *s: _rng.normal(s) * 0.05)(D, Dh)), 'wv': _w((lambda *s: _rng.normal(s) * 0.05)(D, Dh)), 'wo': _w((lambda *s: _rng.normal(s) * 0.05)(H * Dh, D))}
    _A_in = _A_setup()

    def _B_setup():
        B, S, D, F = (1, 2048, 576, 4608)
        return {'x': _w((lambda *s: _rng.normal(s) * 0.05)(B, S, D)), 'w_gate': _w((lambda *s: _rng.normal(s) * 0.05)(D, F)), 'w_up': _w((lambda *s: _rng.normal(s) * 0.05)(D, F)), 'w_down': _w((lambda *s: _rng.normal(s) * 0.05)(F, D))}
    _B_in = _B_setup()
    return {'A_x': _A_in['x'], 'A_wq': _A_in['wq'], 'A_wk': _A_in['wk'], 'A_wv': _A_in['wv'], 'A_wo': _A_in['wo'], 'B_x': _B_in['x'], 'B_w_gate': _B_in['w_gate'], 'B_w_up': _B_in['w_up'], 'B_w_down': _B_in['w_down'], 'c': _w((lambda *s: _rng.normal(s) * 0.05)(1, 576) * 8.0), 'w_mod': _w((lambda *s: _rng.normal(s) * 0.05)(576, 6 * 576) * 576 ** (-0.5) * 8.0)}

def reference(A_x, A_wq, A_wk, A_wv, A_wo, B_x, B_w_gate, B_w_up, B_w_down, c, w_mod):

    def _A_ref(x, wq, wk, wv, wo):
        B, S, D = x.shape
        H = 32
        Dh = D // H
        q = (lambda x, *d: x.transpose(*d))((x @ wq).reshape(B, S, H, Dh), 0, 2, 1, 3)
        k = x @ wk
        v = x @ wv
        scores = jnp.einsum('bhqd,bkd->bhqk', q, k) * Dh ** (-0.5)
        p = _softmax(scores, axis=-1)
        o = jnp.einsum('bhqk,bkd->bhqd', p, v)
        return (lambda x, *d: x.transpose(*d))(o, 0, 2, 1, 3).reshape(B, S, H * Dh) @ wo

    def _B_ref(x, w_gate, w_up, w_down):
        g = _silu(x @ w_gate)
        u = x @ w_up
        return g * u @ w_down
    x = A_x
    mod = (_silu(c) @ w_mod).reshape(c.shape[0], 6, 1, -1)
    sa, ca, ga, sb, cb, gb = (mod[:, 0].copy(), mod[:, 1].copy(), mod[:, 2].copy(), mod[:, 3].copy(), mod[:, 4].copy(), mod[:, 5].copy())
    h = _layernorm(x, axis=-1) * (1 + ca) + sa
    x = x + ga * _A_ref(h, A_wq, A_wk, A_wv, A_wo)
    h = _layernorm(x, axis=-1) * (1 + cb) + sb
    x = x + gb * _B_ref(h, B_w_gate, B_w_up, B_w_down)
    return x
```

```python
import math

import jax
import jax.numpy as jnp
from jax import lax
import jax.experimental.pallas as pl
import jax.experimental.pallas.tpu as pltpu

F32 = jnp.float32
BF16 = jnp.bfloat16
U32 = jnp.uint32

N_HEADS = 32
LN_EPS = 1e-5
LANES = 128
TB = 512
KC = 256
FC = 512
NF = 3
SUM_LO = 2.0 ** -40
SUM_HI = 2.0 ** 80


def _dot(a, b):
    return lax.dot_general(a, b, (((1,), (0,)), ((), ())), preferred_element_type=F32)


def _dot_nt(a, b):
    return lax.dot_general(a, b, (((1,), (1,)), ((), ())), preferred_element_type=F32)


def _tile_lanes(col, n):
    return jnp.concatenate([col] * (n // LANES), axis=1)


def _modulated_layernorm(xT, scale_col, shift_col):
    d, n = xT.shape
    mean = jnp.sum(xT, axis=0, keepdims=True) * (1.0 / d)
    xc = xT - mean
    var = jnp.sum(xc * xc, axis=0, keepdims=True) * (1.0 / d)
    return xc * lax.rsqrt(var + LN_EPS) * _tile_lanes(scale_col, n) + _tile_lanes(shift_col, n)


def _kernel(x_hbm, wq_hbm, wk_hbm, wv_hbm, wo_hbm, wg_hbm, wu_hbm, wd_hbm, c_hbm, wm_hbm,
            out_hbm,
            x_v, wq_v, wk_v, wv_v, wo_v, wg_v, wu_v, wd_v, c_v, wm_v, out_v,
            mod_s, w1_s, wo_s, q_s, k_s, v_s, o_s, x1_s, h2_s, acc_s,
            in_sem, out_sem):
    D, S = x_hbm.shape
    F = wg_hbm.shape[1]
    DH = D // N_HEADS
    NB = S // TB
    TPB = TB // LANES

    copies = {}

    def copy(name, src, dst):
        copies[name] = pltpu.make_async_copy(src, dst, in_sem.at[len(copies)])
        copies[name].start()

    copy("c", c_hbm, c_v)
    copy("wm0", wm_hbm.at[:, pl.ds(0, 2 * D)], wm_v.at[:, pl.ds(0, 2 * D)])
    copy("wq", wq_hbm, wq_v)
    copy("wk", wk_hbm, wk_v)
    copy("wv", wv_hbm, wv_v)
    for b in range(NB):
        copy(("x", b), x_hbm.at[:, pl.ds(b * TB, TB)], x_v.at[b])
    copy("wm1", wm_hbm.at[:, pl.ds(2 * D, 4 * D)], wm_v.at[:, pl.ds(2 * D, 4 * D)])
    copy("wo", wo_hbm, wo_v)
    for j in range(F // FC):
        copy(("wg", j), wg_hbm.at[:, pl.ds(j * FC, FC)], wg_v.at[j])
        copy(("wu", j), wu_hbm.at[:, pl.ds(j * FC, FC)], wu_v.at[j])
        copy(("wd", j), wd_hbm.at[:, pl.ds(j * FC, FC)], wd_v.at[j])

    copies["c"].wait()
    cf = c_v[...].astype(F32)
    sc = jnp.broadcast_to(cf * jax.nn.sigmoid(cf), (16, D)).astype(BF16)

    def modulation(lo, n):
        row = _dot(sc, wm_v[:, lo:lo + n])[0:1]
        mod_s[lo:lo + n, :] = jnp.broadcast_to(row, (LANES, n)).T

    def mod_col(i):
        return mod_s[i * D:(i + 1) * D, :]

    copies["wm0"].wait()
    modulation(0, 2 * D)

    copies["wq"].wait()
    copies["wk"].wait()
    copies["wv"].wait()
    zpad = jnp.zeros((32 - DH, D), F32)
    w1 = jnp.concatenate(
        [wq_v[...].astype(F32).T, wk_v[...].astype(F32), zpad, wv_v[...].astype(F32), zpad], axis=0)
    w1_s[...] = pltpu.bitcast(w1.astype(BF16), U32)
    k_scale = DH ** -0.5 * math.log2(math.e)
    for b in range(NB):
        copies[("x", b)].wait()
        h = _modulated_layernorm(x_v[b].astype(F32), 1.0 + mod_col(1), mod_col(0))
        qkv = _dot(pltpu.bitcast(w1_s[...], BF16), h.astype(BF16))
        q = pltpu.bitcast(qkv[:D].astype(BF16), U32)
        for t in range(TPB):
            q_s[b * TPB + t, 0:D // 2, :] = q[:, t * LANES:(t + 1) * LANES]
            q_s[b * TPB + t, D // 2:, :] = jnp.zeros((8, LANES), U32)
        kT = jnp.concatenate([qkv[D:D + 32] * k_scale, jnp.zeros((LANES - 32, TB), F32)], axis=0)
        k_s[b * TB // 2:(b + 1) * TB // 2, :] = pltpu.bitcast(kT.T.astype(BF16), U32)
        vT = qkv[D + 32:D + 56].astype(BF16).astype(F32)
        is_sum_row = lax.broadcasted_iota(jnp.int32, vT.shape, 0) == DH
        v_s[:, b * TB:(b + 1) * TB] = jnp.where(is_sum_row, 1.0, vT)

    def load_q(hd, b):
        return jnp.concatenate(
            [pltpu.bitcast(q_s[b * TPB + t, pl.ds(hd * (DH // 2), 16), :], BF16) for t in range(TPB)],
            axis=1)

    def load_k(lo, n):
        return pltpu.bitcast(k_s[lo // 2:(lo + n) // 2, :], BF16)[:, :32]

    def store_o(hd, b, acc):
        o = acc / acc[DH:DH + 1]
        for t in range(TPB):
            o_s[b * TPB + t, pl.ds(hd * DH, 24), :] = o[:, t * LANES:(t + 1) * LANES]

    def head_unshifted(hd, unsafe):
        work = [(b, c) for b in range(NB) for c in range(S // KC)]
        pending = None
        acc = None
        for item in work + [None]:
            if item is not None:
                b, c = item
                if c == 0:
                    q = load_q(hd, b)
                p = jnp.exp2(_dot(load_k(c * KC, KC), q)).astype(BF16)
            if pending is not None:
                pb, pc, pp = pending
                part = _dot(v_s[:, pc * KC:(pc + 1) * KC], pp)
                acc = part if pc == 0 else acc + part
                if pc == S // KC - 1:
                    store_o(hd, pb, acc)
                    mag = jnp.maximum(jnp.maximum(jnp.abs(acc[0:8]), jnp.abs(acc[8:16])), jnp.abs(acc[16:24]))
                    ok = (acc[DH:DH + 1] >= SUM_LO) & (mag <= SUM_HI)
                    unsafe = jnp.where(ok, unsafe, 1.0)
            pending = None if item is None else (b, c, p)
        return unsafe

    unsafe = lax.fori_loop(0, N_HEADS, head_unshifted, jnp.zeros((8, TB), F32))

    @pl.when(jnp.max(unsafe) > 0.0)
    def _():
        def head_shifted(i, carry):
            hd = i // NB
            b = i % NB
            s = _dot(load_k(0, S), load_q(hd, b))
            p = jnp.exp2(s - jnp.max(s, axis=0, keepdims=True)).astype(BF16)
            store_o(hd, b, _dot(v_s[...], p))
            return carry

        lax.fori_loop(0, N_HEADS * NB, head_shifted, 0)

    copies["wm1"].wait()
    modulation(2 * D, 4 * D)
    copies["wo"].wait()
    wo_s[...] = pltpu.bitcast(wo_v[...].astype(F32).T.astype(BF16), U32)
    for b in range(NB):
        o = jnp.concatenate([o_s[b * TPB + t, 0:D, :] for t in range(TPB)], axis=1)
        attn = _dot(pltpu.bitcast(wo_s[...], BF16), o.astype(BF16))
        x1 = x_v[b].astype(F32) + _tile_lanes(mod_col(2), TB) * attn
        x1_s[b] = x1
        h2 = _modulated_layernorm(x1, 1.0 + mod_col(4), mod_col(3))
        h2_s[b] = pltpu.bitcast(h2.T.astype(BF16), U32)

    for j in range(F // FC):
        copies[("wg", j)].wait()
        copies[("wu", j)].wait()
        copies[("wd", j)].wait()

    NJ = F // (FC * NF)

    def out_copy(b):
        return pltpu.make_async_copy(
            out_v.at[b], out_hbm.at[:, pl.ds(pl.multiple_of(b * TB, TB), TB)], out_sem.at[b])

    def ffn_block(b, carry):
        acc_s[...] = jnp.zeros_like(acc_s)

        def ffn_step(j, carry):
            h2 = pltpu.bitcast(h2_s[b], BF16)
            acc = None
            prev = None
            for c in range(NF + 1):
                if c < NF:
                    t = 0.5 * _dot(h2, wg_v[j * NF + c])
                    a = ((t + t * jnp.tanh(t)) * _dot(h2, wu_v[j * NF + c])).astype(BF16)
                if prev is not None:
                    y = _dot_nt(wd_v[j * NF + c - 1], prev)
                    acc = y if acc is None else acc + y
                prev = a
            acc_s[...] += acc
            return carry

        lax.fori_loop(0, NJ, ffn_step, 0)
        out_v[b] = (x1_s[b] + _tile_lanes(mod_col(5), TB) * acc_s[...]).astype(out_v.dtype)
        out_copy(b).start()
        return carry

    lax.fori_loop(0, NB, ffn_block, 0)
    for b in range(NB):
        out_copy(b).wait()


@jax.jit
def pallas_adaLN_cond__grouped_kv_mqa__swiglu_ffn__prompt_kernel(
    A_x, A_wq, A_wk, A_wv, A_wo, B_x, B_w_gate, B_w_up, B_w_down, c, w_mod,
):
    del B_x
    _, S, D = A_x.shape
    F = B_w_gate.shape[1]
    DH = D // N_HEADS
    NB = S // TB
    NC = F // FC
    dt = A_x.dtype
    vmem = pltpu.VMEM
    scratch = [
        vmem((NB, D, TB), dt), vmem((D, D), dt), vmem((DH, D), dt), vmem((DH, D), dt), vmem((D, D), dt),
        vmem((NC, D, FC), dt), vmem((NC, D, FC), dt), vmem((NC, D, FC), dt),
        vmem((1, D), dt), vmem((D, 6 * D), dt), vmem((NB, D, TB), dt),
        vmem((6 * D, LANES), F32),
        vmem(((D + 64) // 2, D), U32),
        vmem((D // 2, D), U32),
        vmem((S // LANES, D // 2 + 8, LANES), U32),
        vmem((S // 2, LANES), U32),
        vmem((24, S), F32),
        vmem((S // LANES, D + 8, LANES), F32),
        vmem((NB, D, TB), F32),
        vmem((NB, TB // 2, D), U32),
        vmem((D, TB), F32),
        pltpu.SemaphoreType.DMA((7 + NB + 3 * NC,)),
        pltpu.SemaphoreType.DMA((NB,)),
    ]
    outT = pl.pallas_call(
        _kernel,
        out_shape=jax.ShapeDtypeStruct((D, S), dt),
        in_specs=[pl.BlockSpec(memory_space=pl.ANY)] * 10,
        out_specs=pl.BlockSpec(memory_space=pl.ANY),
        scratch_shapes=scratch,
        compiler_params=pltpu.CompilerParams(vmem_limit_bytes=110 * 1024 * 1024),
        name="adaln_mqa_swiglu",
    )(A_x[0].T, A_wq, A_wk.T, A_wv.T, A_wo, B_w_gate, B_w_up, B_w_down.T, c, w_mod)
    return outT.T[None]
```

```python
import contextlib
import itertools
import math

import jax
import jax.numpy as jnp
import numpy as np
from jax import lax
import jax.experimental.pallas as pl
import jax.experimental.pallas.tpu as pltpu

F32 = jnp.float32
BF16 = jnp.bfloat16
U32 = jnp.uint32

N_HEADS = 32
LN_EPS = 1e-5
T = 128
TB = 512
FU = 512
MH = 64
VPU_GROUPS = (1, 2, 1, 2, 2, 1, 2, 1, 2, 1, 2, 1, 2, 1, 2, 0)
AHEAD = 8
HEADS_PER_STEP = 2
SUM_MIN = 2.0 ** -30
SUM_MAX = 2.0 ** 120
R3 = math.sqrt(3.0)

PROFILE = False
ONLY = None
HEAD_SLOTS = 3
DELAY = 2
DOWN_AT = 1
LAG = 2
GU_START = 2
PREP_L1 = 0
E0 = 0
E1 = 1.6
X1_OPAQUE = False
SMODE = 0


def _scope(name):
    return jax.named_scope(name) if PROFILE else contextlib.nullcontext()


def _gate_up_scheme():
    e = [[np.outer(np.eye(2)[i], np.eye(2)[j]) for j in range(2)] for i in range(2)]
    alpha = [e[0][0] + e[1][1], e[1][0] + e[1][1], e[0][0], e[1][1],
             e[0][0] + e[0][1], e[1][0] - e[0][0], e[0][1] - e[1][1]]
    beta = [e[0][0] + e[1][1], e[0][0], e[0][1] - e[1][1], e[1][0] - e[0][0],
            e[1][1], e[0][0] + e[0][1], e[1][0] + e[1][1]]
    gamma = [e[0][0] + e[1][1], e[1][0] - e[1][1], e[0][1] + e[1][1], e[0][0] + e[1][0],
             e[0][1] - e[0][0], e[1][1], e[0][0]]

    def inv(m):
        return np.array([[m[1, 1], -m[0, 1]], [-m[1, 0], m[0, 0]]]) / (m[0, 0] * m[1, 1] - m[0, 1] * m[1, 0])

    def frame(p1, p2, p3):
        m = np.array([p1, p2], float).T
        return m * (inv(m) @ np.array(p3, float))

    u1, u2, u3, u4 = (1, 1), (-2, 1), (1, 0), (0, 1)
    w1, w2, w2p, w3, w4 = (1, 1), (-2, 1), (1, -2), (1, 0), (0, 1)
    products = []
    bases = [((u1, u2, u3), (w1, w2, w3)), ((u1, u2, u4), (w1, w2, w4)),
             ((u1, u2, u3), (w1, w2p, w4)), ((u1, u2, u4), (w1, w2p, w3))]
    for n, (us, ws) in enumerate(bases):
        left = frame(*us)
        t = frame(ws[1], ws[0], ws[2])
        right = np.array([t[:, 0], -t[:, 1]])
        for al, be, ga in zip(alpha, beta, gamma):
            a, b = np.zeros((2, 9)), np.zeros((9, 2))
            a[:, 2 * n:2 * n + 2] = inv(left).T @ al
            b[2 * n:2 * n + 2] = be @ inv(right).T
            products.append((a, b, left @ ga @ right))
    for i, u in enumerate((u3, u4)):
        for j, w in enumerate((w2, w2p)):
            a, b = np.zeros((2, 9)), np.zeros((9, 2))
            a[i, 8] = 1.0
            b[8] = inv(np.array([w2, w2p], float))[:, j]
            products.append((a, b, np.outer(u, w)))
    o = np.outer
    patterns = [o(u2, w1), o(u2, w1), o(u3, w1), o(u4, w1),
                o(u1, w2), o(u3, w2), o(u4, w2), np.array([[0, 1], [-1, 0]]),
                o(u1, w2p), o(u3, w2p), o(u4, w2p), np.array([[1, 0], [0, -1]]),
                o(u1, w3), o(u2, w3), o(u1, w4), o(u2, w4)]
    passes = [[] for _ in patterns]
    for a, b, g in products:
        for couple, pattern in zip(passes, patterns):
            s = (g * pattern).sum() / (pattern * pattern).sum()
            if len(couple) < 2 and np.allclose(g, s * pattern):
                lead = b.flat[np.argmax(np.abs(b) > 1e-9)]
                couple.append((np.round(a * s * lead, 12), np.round(b / lead, 12)))
                break
    assert all(len(couple) == 2 for couple in passes)
    return passes


GATE_UP_PASSES = _gate_up_scheme()


def _gate_up_combine(four_passes):
    m = four_passes(0)
    x = m[0] + m[1]
    p = [m[2] - (x + x), m[3] + x]
    m = four_passes(1)
    q = [m[0] + m[1], m[0] + m[2]]
    c = [[(p[i] - q[i]) - q[i], p[i] + q[i]] for i in range(2)]
    c[0][1] += m[3]
    c[1][0] -= m[3]
    m = four_passes(2)
    q = [m[0] + m[1], m[0] + m[2]]
    c = [[c[i][0] + q[i], (c[i][1] - q[i]) - q[i]] for i in range(2)]
    c[0][0] += m[3]
    c[1][1] -= m[3]
    m = four_passes(3)
    return [[c[0][0] + (m[0] - (m[1] + m[1])), c[0][1] + (m[2] - (m[3] + m[3]))],
            [c[1][0] + (m[0] + m[1]), c[1][1] + (m[2] + m[3])]]


def _lincomb(coef, block):
    groups = {}
    for idx in np.argwhere(coef != 0):
        c = float(coef[tuple(idx)])
        v = block(*(int(i) for i in idx))
        if abs(c) in groups:
            g = groups[abs(c)]
            g[1] = g[1] + v if g[0] == c else g[1] - v
        else:
            groups[abs(c)] = [c, v]
    acc = None
    for c, v in groups.values():
        if acc is not None and c == -1.0:
            acc = acc - v
        else:
            v = v if c == 1.0 else v * c
            acc = v if acc is None else acc + v
    return acc


def _strassen_lhs(w):
    f, e = w[0][0] - w[1][1], w[1][0] - w[0][1]
    return [f, f + e, w[0][0] + w[0][1], w[0][1] + w[1][1], w[0][0] - w[0][1], e - f, w[1][1] - w[0][1]]


def _strassen_rhs(x):
    f, e = x[0][1] - x[1][0], x[1][1] - x[0][0]
    return [f, x[0][1] - x[0][0], x[0][0] + x[1][0], f + e, x[0][0] - x[1][0], x[0][0] + x[0][1], f - e]


def _strassen_out(m):
    s = m[2] + m[4]
    d = (m[2] - m[4]) + (m[0] + m[0])
    return [[s, d + (m[3] + m[6])], [d + (m[5] - m[1]), s + (m[5] + m[1]) + (m[3] - m[6])]]


def _dot(a, b):
    return lax.dot_general(a, b, (((1,), (0,)), ((), ())), preferred_element_type=F32)


def _dot_nt(a, b):
    return lax.dot_general(a, b, (((1,), (1,)), ((), ())), preferred_element_type=F32)


def _pack(x):
    return pltpu.bitcast(x.astype(BF16), U32)


def _unpack(x):
    return pltpu.bitcast(x, BF16)


def _vregs(x):
    return [x[i:i + 8] for i in range(0, x.shape[0], 8)]


def _moments(x, progress=None):
    s1 = x - x[0:1]
    s2 = s1 * s1
    if progress is not None:
        s1, s2 = (list(itertools.accumulate(_vregs(z))) for z in (s1, s2))
        progress += itertools.chain(*zip(s1[2::6], s2[5::6]))
        s1, s2 = s1[-1], s2[-1]
    mean = jnp.sum(s1, axis=0, keepdims=True) * (1.0 / x.shape[0])
    var = jnp.sum(s2, axis=0, keepdims=True) * (1.0 / x.shape[0]) - mean * mean
    return x[0:1] + mean, lax.rsqrt(jnp.maximum(var, 0.0) + LN_EPS)


def _after(always, x, deps):
    if not deps:
        return x
    z = pltpu.bitcast(deps[0], U32)
    for d in deps[1:]:
        z = z | pltpu.bitcast(d, U32)
    mask = jnp.concatenate([always[:, :x.shape[1]]] * (x.shape[0] // 8), axis=0) != 0
    return jnp.where(mask, x, z[:, :x.shape[1]])


def _after_each(always, x, deps):
    parts = []
    for busy, run in itertools.groupby(enumerate(deps), key=lambda e: bool(e[1])):
        run = list(run)
        if busy:
            parts += [_after(always, x[8 * i:8 * i + 8], d) for i, d in run]
        else:
            parts.append(x[8 * run[0][0]:8 * run[-1][0] + 8])
    return jnp.concatenate(parts, axis=0)


class _Spread:
    def __init__(self, items, count, stop, start=0):
        self.items, self.count, self.slots = iter(items), count, stop - start
        self.now, self.done = -start, 0

    def advance(self, dt):
        self.now += dt
        out = []
        while self.done < min(self.count, self.now * self.count // self.slots):
            self.done += 1
            out.append(next(self.items))
        return out


def _kernel(x_hbm, wq_hbm, wk_hbm, wv_hbm, wo_hbm, wg_hbm, wu_hbm, wd_hbm, c_hbm, wm_hbm,
            out_hbm,
            x_v, wq_v, wk_v, wv_v, wo_v, wg_v, wu_v, wd_v, c_v, wm_v, out_v,
            mod_s, wqkv_s, wo_s, q_s, kvs_s, kb_s, o_s, x1_s, h2_s, wgu_s, wd_s, act_s, acc_s,
            zero_s, in_sem, out_sem):
    D, S = x_hbm.shape
    F = wg_hbm.shape[1]
    DH = D // N_HEADS
    NB = S // TB
    TPB = TB // T
    NK = S // T
    NU = F // FU
    KS = D // 9
    RB = D // 4
    n_mxu = [T // 16 - n for n in VPU_GROUPS]
    g_off = [2 * sum(VPU_GROUPS[:c]) for c in range(NK + 1)]
    NG = g_off[-1]
    V0 = S // 16
    S0 = V0 + 3 * NK

    def score_at(tile, g):
        return S0 + tile * NG + g

    def mod(i):
        return mod_s[i * D:(i + 1) * D, :]

    def all_true():
        return pltpu.bitcast(mod_s[0:8, :], U32) | 1

    def project(w_ref, tiles, *side):
        always = all_true()
        nrow = w_ref.shape[0] // 8
        side = [_Spread(items, count, nrow * 5 * TPB) for items, count in side]

        def lhs(lanes, dt):
            deps = [[[y for s in side for y in s.advance(dt)] for _ in lanes] for _ in range(nrow)]
            return [_unpack(_after_each(always, w_ref[:, ds], d)) for ds, d in zip(lanes, zip(*deps))]

        main = []
        for z in tiles:
            m = [_dot(w, z[j * T:(j + 1) * T].astype(BF16))
                 for j, w in enumerate(lhs([pl.ds(j * T, T) for j in range(4)], 1))]
            main.append((m[0] + m[1]) + (m[2] + m[3]))
        w, = lhs([pl.ds(4 * T, D - 4 * T)], TPB)
        return [m + _dot(w, z[4 * T:].astype(BF16)) for m, z in zip(main, tiles)]

    copies = {}

    def copy(name, src, dst):
        copies[name] = pltpu.make_async_copy(src, dst, in_sem.at[len(copies)])
        copies[name].start()

    def wait(*names):
        with _scope("wait_" + str(names[0])):
            for name in names:
                copies[name].wait()

    copy("c", c_hbm, c_v)
    copy("wm0", wm_hbm.at[:, pl.ds(0, 2 * D)], wm_v.at[:, pl.ds(0, 2 * D)])
    copy("wq", wq_hbm, wq_v)
    copy("wk", wk_hbm, wk_v)
    copy("wv", wv_hbm, wv_v)
    for b in range(NB):
        copy(("x", b), x_hbm.at[:, pl.ds(b * TB, TB)], x_v.at[b])

    def clear(i, carry):
        acc_s[i // 7, pl.ds(i % 7 * 7, 7)] = jnp.zeros((7, RB, T), F32)
        return carry

    zero_s[0] = 0
    lax.fori_loop(0, 7 * NB, clear, 0)

    def modulation(lo, n):
        cf = c_v[...].astype(F32)
        sc = jnp.broadcast_to(cf * jax.nn.sigmoid(cf), (16, D)).astype(BF16)
        row = _dot(sc, wm_v[:, lo:lo + n])[0:1]
        col = lo + lax.broadcasted_iota(jnp.int32, (1, n), 1)
        is_scale = ((col >= D) & (col < 2 * D)) | ((col >= 4 * D) & (col < 5 * D))
        mod_s[lo:lo + n, :] = jnp.broadcast_to(jnp.where(is_scale, 1.0 + row, row), (T, n)).T

    wait("c", "wm0")
    modulation(0, 2 * D)

    wait("wq", "wk", "wv")
    pad = jnp.zeros((24 - DH, D), F32)
    wqkv_s[0:24, :] = _pack(jnp.concatenate([wk_v[...].astype(F32), pad, wv_v[...].astype(F32), pad], axis=0))
    wqkv_s[24:, :] = pltpu.bitcast(wq_v[...].T, U32)
    vpu_keys = []

    def project_qkv(b, *side):
        h = []
        for t in range(TPB):
            x = x_v[b, :, t * T:(t + 1) * T].astype(F32)
            mean, rstd = _moments(x)
            h.append((x - mean) * rstd * mod(1) + mod(0))
        done = []
        for t, y in enumerate(project(wqkv_s, h, *side)):
            c = b * TPB + t
            q_s[c, 0:D, :] = y[48:]
            q_s[c, D:, :] = jnp.zeros((32, T), F32)
            k = y[0:24] * (DH ** -0.5 * math.log2(math.e))
            k = jnp.concatenate([k, jnp.zeros((T - 24, T), F32)], axis=0).T
            kvs_s[8 * c:8 * c + 8] = pltpu.bitcast(k.astype(BF16), F32).reshape(8, 8, T)
            is_sum_row = lax.broadcasted_iota(jnp.int32, (24, T), 0) == DH
            kvs_s[V0 + 3 * c:V0 + 3 * c + 3] = jnp.where(is_sum_row, 1.0, y[24:48]).reshape(3, 8, T)
            if VPU_GROUPS[c]:
                vpu_keys.append(k[n_mxu[c] * 16:])
                for d in range(DH):
                    kb = jnp.broadcast_to(vpu_keys[-1][:, d:d + 1], vpu_keys[-1].shape)
                    kb_s[g_off[c]:g_off[c + 1], d] = kb.reshape(-1, 8, T)
                    done += _vregs(kb)
        return done, len(done)

    wait(("x", 0))
    project_qkv(0)
    wait(*[("x", b) for b in range(1, NB)])
    copy("wm1", wm_hbm.at[:, pl.ds(2 * D, 4 * D)], wm_v.at[:, pl.ds(2 * D, 4 * D)])
    copy("wo", wo_hbm, wo_v)
    copy("fence", wk_hbm, wk_v)
    for u in range(NU):
        copy(("wg", u), wg_hbm.at[:, pl.ds(u * FU, FU)], wg_v.at[u])
        copy(("wu", u), wu_hbm.at[:, pl.ds(u * FU, FU)], wu_v.at[u])
        copy(("wd", u), wd_hbm.at[:, pl.ds(u * FU, FU)], wd_v.at[u])
    project_qkv(3, project_qkv(2, project_qkv(1)))

    for t in range(TPB):
        kvs_s[score_at(t, 0):score_at(t, NG)] = _dot(
            jnp.concatenate(vpu_keys, axis=0)[:, :32].astype(BF16),
            q_s[t, 0:32, :].astype(BF16)).reshape(NG, 8, T)

    def attend_unshifted(step, safe):
        zero = zero_s[0]

        def vpu_scores(head, b):
            for tile in range(b * TPB, (b + 1) * TPB):
                q = q_s[tile, pl.ds(head * DH, 24), :]
                q = [jnp.broadcast_to(q[d:d + 1], (8, T)) for d in range(DH)]
                span = SMODE or NG
                for g0 in range(0, NG, span):
                    s = [None, None]
                    for d in range(DH):
                        z = kb_s[g0:min(NG, g0 + span), d] * q[d]
                        s[d % 2] = z if d < 2 else s[d % 2] + z
                    s = s[0] + s[1]
                    for g in range(s.shape[0]):
                        kvs_s[zero + score_at(tile, g0 + g)] = s[g]
                        yield

        cols = [(step * HEADS_PER_STEP + n // NB, n % NB) for n in range(HEADS_PER_STEP * NB + 1)]
        side = itertools.chain(*[vpu_scores(*col) for col in cols[1:]])
        cols.pop()
        groups = [(n, c, r) for n in range(len(cols)) for c in range(NK) for r in reversed(range(n_mxu[c]))]
        side = _Spread(side, len(cols) * TPB * NG, 2 * len(groups) + 3 * len(cols) * NK, HEAD_SLOTS)

        def load(idx, dt):
            side.advance(dt)
            return kvs_s[idx]

        q = [jnp.concatenate([q_s[b * TPB + t, pl.ds(head * DH, 32), :] for t in range(TPB)],
                             axis=1).astype(BF16) for head, b in cols]
        p = {}
        pos = end = 0
        for n, (head, b) in enumerate(cols):
            acc = None
            for c in range(NK):
                rows = []
                if VPU_GROUPS[c]:
                    rows = [jnp.exp2(jnp.concatenate(
                        [kvs_s[score_at(b * TPB + t, g_off[c]):score_at(b * TPB + t, g_off[c + 1])].reshape(-1, T)
                         for t in range(TPB)], axis=1))]
                end += n_mxu[c]
                while pos < min(end + AHEAD, len(groups)):
                    run = [g for g in groups[pos:end + AHEAD] if g[0] == groups[pos][0]]
                    k = jnp.concatenate([load(8 * cc + r, 2) for _, cc, r in run], axis=0)
                    e = jnp.exp2(_dot(_unpack(k)[:, :32], q[run[0][0]]))
                    p.update((g, e[16 * j:16 * j + 16]) for j, g in enumerate(run))
                    pos += len(run)
                rows = [p.pop((n, c, r)) for r in range(n_mxu[c])] + rows
                v = jnp.concatenate([load(V0 + 3 * c + r, 1) for r in range(3)], axis=0)
                part = _dot(v, jnp.concatenate(rows, axis=0))
                acc = part if acc is None else acc + part
            for t in range(TPB):
                total = jnp.broadcast_to(acc[DH:DH + 1, t * T:(t + 1) * T], (8, T))
                inv = pltpu.reciprocal(total, approx=True)
                inv = inv * (2.0 - total * inv)
                o = [z * inv for z in _vregs(acc[:, t * T:(t + 1) * T])]
                o_s[b * TPB + t, pl.ds(head * DH, 24), :] = jnp.concatenate(o, axis=0)
                probe = (o[0] + o[1]) + (o[2] + total)
                safe = jnp.where((total >= SUM_MIN) & (jnp.abs(probe) <= SUM_MAX), safe, 0.0)
        assert side.done == side.count
        return safe

    safe = jnp.ones((8, T), F32)
    with _scope("attn"):
        if ONLY in ("early", "ffn"):
            safe = kvs_s[S0]
        else:
            safe = lax.fori_loop(0, N_HEADS // HEADS_PER_STEP, attend_unshifted, safe)

    @pl.when(jnp.min(safe) < 1.0)
    def _():
        def attend_shifted(i, carry):
            head, tile = i // NK, i % NK
            k = _unpack(kvs_s[0:V0].reshape(S // 2, T))[:, :32]
            v = jnp.concatenate([kvs_s[V0 + 3 * c:V0 + 3 * c + 3].reshape(24, T) for c in range(NK)], axis=1)
            s = _dot(k, q_s[tile, pl.ds(head * DH, 32), :].astype(BF16))
            acc = _dot(v, jnp.exp2(s - jnp.max(s, axis=0, keepdims=True)).astype(BF16))
            o_s[tile, pl.ds(head * DH, 24), :] = acc / acc[DH:DH + 1]
            return carry

        lax.fori_loop(0, N_HEADS * NK, attend_shifted, 0)

    wait("wm1", "wo", *[(name, u) for u in range(NU) for name in ("wg", "wu", "wd")])
    if ONLY == "attn":
        wait("fence")
        out_v[0] = jnp.concatenate([o_s[t, 0:D, :] for t in range(TPB)], axis=1).astype(BF16)
        cp = pltpu.make_async_copy(out_v.at[0], out_hbm.at[:, pl.ds(0, TB)], out_sem.at[0])
        cp.start()
        cp.wait()
        return
    wo_s[...] = pltpu.bitcast(wo_v[...].T, U32)
    modulation(2 * D, 4 * D)
    tile_scale = [math.sqrt(R3 ** ((1 - i) + s)) for i in range(2) for s in range(2)]

    def project_out(b, *side):
        attn = project(wo_s, [o_s[b * TPB + t, 0:D, :] for t in range(TPB)], *side)
        for t in range(TPB):
            x1_s[zero_s[0] + b if X1_OPAQUE else b, t] = x_v[b, :, t * T:(t + 1) * T].astype(F32) + mod(2) * attn[t]

        progress = []
        stats = [_moments(x1_s[b, t], progress) for t in range(TPB)]

        def operands(start):
            h2 = []
            for t, (mean, rstd) in enumerate(stats):
                mean = pltpu.bitcast(jnp.broadcast_to(mean, (8, T)), U32)
                mean = pltpu.bitcast(_after(all_true(), mean, [start()]), F32)[0:1]
                z = (x1_s[b, t] - mean) * (rstd * tile_scale[t]) * mod(4)
                h2.append(z + (mod(3) if tile_scale[t] == 1.0 else mod(3) * tile_scale[t]))
            for s in range(2):
                for r, couple in enumerate(GATE_UP_PASSES):
                    z = [_lincomb(a, lambda i, k: h2[2 * i + s][k * KS:(k + 1) * KS]) for a, _ in couple]
                    z = pltpu.bitcast(jnp.concatenate(z, axis=0).astype(BF16).T, U32)
                    h2_s[b, r, s * T // 2:(s + 1) * T // 2, :] = z
                    yield from _vregs(z)[1::2]

        return (progress, len(progress)), lambda start: (operands(start), 2 * 16 * T // 32)

    def prepare_gate_up(u, t):
        terms = sorted(((int(np.argwhere(coef != 0)[0, 0]) // 2, r, m, coef)
                        for r, couple in enumerate(GATE_UP_PASSES) for m, (_, coef) in enumerate(couple)),
                       key=lambda e: e[:3])

        def work():
            for n, w_v in enumerate((wg_v, wu_v)):
                w = [w_v[u, :, pl.ds((2 * j + t) * T, T)].astype(F32) for j in range(2)]
                done = []
                for _, r, m, coef in terms:
                    done.append(_pack(_lincomb(coef, lambda k, j: w[j][k * KS:(k + 1) * KS])))
                for i in range(KS // 16):
                    for (_, r, m, _), y in zip(terms, done):
                        wgu_s[2 * t + n, r, pl.ds(m * KS // 2 + 8 * i, 8), :] = y = y[8 * i:8 * i + 8]
                        yield y

        return work(), 2 * 16 * T // 16

    def prepare_down(u):
        def work():
            def block(r1, r2, j, t):
                w = wd_v[u, pl.ds((2 * r1 + r2) * RB, RB), pl.ds((2 * j + t) * T, T)].astype(F32)
                return w if r1 + r2 == j + t else w * R3 ** (r1 + r2 - j - t)

            outer = [[_strassen_lhs([[block(r1, r2, j, t) for j in range(2)] for r1 in range(2)])
                      for t in range(2)] for r2 in range(2)]
            done = [_pack(y) for r in range(7)
                    for y in _strassen_lhs([[outer[r2][t][r] for t in range(2)] for r2 in range(2)])]
            for r, y in enumerate(done):
                wd_s[r] = y
            for i in range(RB // 16):
                if PREP_L1:
                    yield from (z[16 * i + k:16 * i + k + 8] for row in outer for forms in row for z in forms
                                for k in (0, 8))
                yield from (y[8 * i:8 * i + 8] for y in done)

        return work(), (49 + 56 * PREP_L1) * RB // 16

    def finish(b, inner):
        def work():
            for r2 in range(2):
                for s in range(2):
                    y = _strassen_out([inner[r][r2][s] for r in range(7)])
                    done = []
                    for r1 in range(2):
                        for i in range(2):
                            rows = pl.ds((2 * r1 + r2) * RB, RB)
                            tile = 2 * (1 - i) + s
                            gate = mod_s[pl.ds(5 * D + (2 * r1 + r2) * RB, RB), :] * (0.125 * R3 ** -(r1 + r2 + i + s))
                            z = x1_s[b, tile, rows, :] + gate * y[r1][i]
                            out_v[b, rows, pl.ds(tile * T, T)] = z.astype(out_v.dtype)
                            done.append(_vregs(z))
                    yield from itertools.chain(*zip(*done))

        return work(), TPB * D // 8

    slabs = TB // (2 * MH)

    class Ffn:
        def __init__(self):
            self.always = all_true()
            self.side = []
            self.due = []

        def run_under(self, work, stop, start=0):
            slots = 2 * 16 * TB // 32
            self.side.append(_Spread(*work, int(stop * slots), int(start * slots)))

        def lhs(self, x, due, side):
            due = [z.reshape(-1, 2, 8, T) for z in due]
            x = _after(self.always, x, [z[:, k].reshape(x.shape) for z in due for k in range(2)])
            return _unpack(_after_each(self.always, x, [[y for s in side for y in s.advance(1)]
                                                        for _ in range(x.shape[0] // 8)]))

        def next_round(self, rows):
            self.due = [(n - 1, z) for n, z in self.due]
            now = [z for n, z in self.due if n < 0 and z.shape[0] == rows]
            self.due = [(n, z) for n, z in self.due if n >= 0 or z.shape[0] != rows]
            return now

        def product(self, b, n, slab):
            def four_passes(k):
                due = self.next_round(MH)
                return [_dot(self.lhs(h2_s[b, 4 * k + r, pl.ds(slab * MH // 2, MH // 2), :], due[r::4], self.side),
                             _unpack(wgu_s[n, 4 * k + r])) for r in range(4)]

            return _gate_up_combine(four_passes)

        def gate_up(self, b, t, midway=None, at=None):
            parts = []
            for slab in range(slabs):
                g = self.product(b, 2 * t, slab)

                def silu2(i, j):
                    th = jnp.tanh(g[i][j] * (0.5 / tile_scale[2 * i + slab * MH // T]))
                    z = g[i][j] if j + t == 0 else g[i][j] * R3 ** (j + t)
                    return z + z * th

                act = [[silu2(i, j) for j in range(2)] for i in range(2)]
                self.due += [(DELAY, z) for z in act[0] + act[1]]
                up = self.product(b, 2 * t + 1, slab)
                parts.append(_strassen_rhs([[act[1 - i][j] * up[1 - i][j] for i in range(2)] for j in range(2)]))
                self.due += [(DELAY, z) for z in parts[-1]]
                if midway is not None and slab == (DOWN_AT if at is None else at):
                    midway()
            return [jnp.concatenate(z, axis=0) for z in zip(*parts)]

        def first_half(self, b, midway=None):
            for r, z in enumerate(self.gate_up(b, 0, midway)):
                act_s[b, r] = z

        def second_half(self, b, midway, last=False, at=None):
            outer = [[act_s[b, r] for r in range(7)], self.gate_up(b, 1, midway, at)]

            def down():
                rhs = [y for r in range(7)
                       for y in _strassen_rhs([[outer[t][r][:T], outer[t][r][T:]] for t in range(2)])]
                inner = []
                for r in range(49):
                    if r % 4 == 0:
                        due = self.next_round(RB)
                    y = acc_s[b, r] + _dot_nt(self.lhs(wd_s[r], due[r % 4::4], []), rhs[r].astype(BF16))
                    if not last:
                        acc_s[b, r] = y
                        continue
                    inner.append(y)
                    if r % 7 == 6:
                        inner[-7:] = [_strassen_out(inner[-7:])]
                        self.due += [(1, z) for z in inner[-1][0] + inner[-1][1]]
                if last:
                    self.due = [(n, z) for n, z in self.due if z.shape[0] != RB]
                    self.run_under(finish(b, inner), 0.75, 0.05)

            return down

    norm0, operands0 = project_out(0, prepare_gate_up(0, 0))
    norm1, operands1 = project_out(1, norm0, prepare_gate_up(0, 1))
    norm2, operands2 = project_out(2, norm1, operands0(lambda: x1_s[1, 0, 0:8]))
    norm3, operands3 = project_out(3, norm2, operands1(lambda: x1_s[2, 0, 0:8]))
    ffn = Ffn()
    ffn.run_under(norm3, E1, E0)
    ffn.run_under(operands2(lambda: x1_s[3, 0, 0:8]), E1)
    ffn.run_under(operands3(lambda: act_s[0, 0, TB // 2 - 8:]), 3, E1)
    for b in range(NB):
        ffn.first_half(b)

    def unit(u, carry):
        ffn = Ffn()
        ffn.run_under(prepare_down(u), LAG + (DOWN_AT + 1) / slabs)
        ffn.run_under(prepare_gate_up(u + 1, 0), NB, GU_START)
        downs = [None] * LAG
        for b in range(NB):
            downs.append(ffn.second_half(b, downs.pop(0)))
        ffn.run_under(prepare_gate_up(u + 1, 1), NB, 0.05)
        for b in range(NB):
            ffn.first_half(b, downs.pop(0) if downs else None)
        return carry

    if ONLY == "early":
        wait("fence")
        def keep(i, c):
            out_v[0, 0:64, 0:T] = (act_s[i, i, 0:64] + pltpu.bitcast(wgu_s[i, i] | h2_s[i, i, 0:64], F32) + x1_s[i, i, 0:64]).astype(BF16)
            return c
        lax.fori_loop(0, 4, keep, 0)
        cp = pltpu.make_async_copy(out_v.at[0], out_hbm.at[:, pl.ds(0, TB)], out_sem.at[0])
        cp.start()
        cp.wait()
        return
    with _scope("units"):
        lax.fori_loop(0, NU - 1, unit, 0)

    def out_copy(b):
        return pltpu.make_async_copy(out_v.at[b], out_hbm.at[:, pl.ds(b * TB, TB)], out_sem.at[b])

    ffn = Ffn()
    ffn.run_under(prepare_down(NU - 1), 1.75)
    down = None
    for b in range(NB):
        down = ffn.second_half(b, down, last=True, at=NB - 1 - b)
    assert all(s.done == s.count for s in ffn.side)
    for b in range(NB - 1):
        out_copy(b).start()
    wait("fence")
    down()
    ffn.side[-1].advance(ffn.side[-1].slots * 2)
    out_copy(NB - 1).start()
    with _scope("out_wait"):
        for b in range(NB):
            out_copy(b).wait()


@jax.jit
def pallas_adaLN_cond__grouped_kv_mqa__swiglu_ffn__prompt_kernel(
    A_x: jax.Array,
    A_wq: jax.Array,
    A_wk: jax.Array,
    A_wv: jax.Array,
    A_wo: jax.Array,
    B_x: jax.Array,
    B_w_gate: jax.Array,
    B_w_up: jax.Array,
    B_w_down: jax.Array,
    c: jax.Array,
    w_mod: jax.Array,
):
    del B_x
    B, S, D = A_x.shape
    F = B_w_gate.shape[1]
    assert (B, S, D) == (1, T * len(VPU_GROUPS), 576) and F % FU == 0 and A_x.dtype == BF16
    DH = D // N_HEADS
    NB, NU, NK = S // TB, F // FU, S // T
    NG = 2 * sum(VPU_GROUPS)
    vmem = pltpu.VMEM
    scratch = [
        vmem((NB, D, TB), BF16),
        vmem((D, D), BF16),
        vmem((DH, D), BF16),
        vmem((DH, D), BF16),
        vmem((D, D), BF16),
        vmem((NU, D, FU), BF16),
        vmem((NU, D, FU), BF16),
        vmem((NU, D, FU), BF16),
        vmem((1, D), BF16),
        vmem((D, 6 * D), BF16),
        vmem((NB, D, TB), BF16),
        vmem((6 * D, T), F32),
        vmem(((D + 48) // 2, D), U32),
        vmem((D // 2, D), U32),
        vmem((NK, D + 32, T), F32),
        vmem((S // 16 + 3 * NK + NK * NG, 8, T), F32),
        vmem((NG, DH, 8, T), F32),
        vmem((NK, D + 8, T), F32),
        vmem((NB, TB // T, D, T), F32),
        vmem((NB, 16, TB // 4, T), U32),
        vmem((4, 16, T // 2, T), U32),
        vmem((49, D // 8, T), U32),
        vmem((NB, 7, TB // 2, T), F32),
        vmem((NB, 49, D // 4, T), F32),
        pltpu.SMEM((1,), jnp.int32),
        pltpu.SemaphoreType.DMA((8 + NB + 3 * NU,)),
        pltpu.SemaphoreType.DMA((NB,)),
    ]
    out = pl.pallas_call(
        _kernel,
        out_shape=jax.ShapeDtypeStruct((D, S), BF16),
        in_specs=[pl.BlockSpec(memory_space=pl.ANY)] * 10,
        out_specs=pl.BlockSpec(memory_space=pl.ANY),
        scratch_shapes=scratch,
        compiler_params=pltpu.CompilerParams(vmem_limit_bytes=110 * 1024 * 1024),
        name="adaln_mqa_swiglu",
    )(A_x[0].T, A_wq, A_wk.T, A_wv.T, A_wo, B_w_gate, B_w_up, B_w_down.T, c, w_mod)
    return out.T[None]
```

```python
import functools
import itertools
import math

import jax
import jax.numpy as jnp
import numpy as np
from jax import lax
import jax.experimental.pallas as pl
import jax.experimental.pallas.tpu as pltpu

F32 = jnp.float32
BF16 = jnp.bfloat16
U32 = jnp.uint32

N_HEADS = 32
LN_EPS = 1e-5
T = 128
TB = 512
FU = 512
MH = 64
VPU_GROUPS = (1, 2, 1, 2, 2, 1, 2, 2, 1, 2, 2, 1, 2, 1, 1, 0)
AHEAD = 8
HEADS_PER_STEP = 2
SUM_MIN = 2.0 ** -30
SUM_MAX = 2.0 ** 120
R3 = math.sqrt(3.0)


def _gate_up_scheme():
    e = [[np.outer(np.eye(2)[i], np.eye(2)[j]) for j in range(2)] for i in range(2)]
    alpha = [e[0][0] + e[1][1], e[1][0] + e[1][1], e[0][0], e[1][1],
             e[0][0] + e[0][1], e[1][0] - e[0][0], e[0][1] - e[1][1]]
    beta = [e[0][0] + e[1][1], e[0][0], e[0][1] - e[1][1], e[1][0] - e[0][0],
            e[1][1], e[0][0] + e[0][1], e[1][0] + e[1][1]]
    gamma = [e[0][0] + e[1][1], e[1][0] - e[1][1], e[0][1] + e[1][1], e[0][0] + e[1][0],
             e[0][1] - e[0][0], e[1][1], e[0][0]]

    def inv(m):
        det = m[0, 0] * m[1, 1] - m[0, 1] * m[1, 0]
        return np.array([[m[1, 1], -m[0, 1]], [-m[1, 0], m[0, 0]]]) / det

    def frame(p1, p2, p3):
        m = np.array([p1, p2], float).T
        return m * (inv(m) @ np.array(p3, float))

    u1, u2, u3, u4 = (1, 1), (-2, 1), (1, 0), (0, 1)
    w1, w2, w2p, w3, w4 = (1, 1), (-2, 1), (1, -2), (1, 0), (0, 1)
    products = []
    bases = [((u1, u2, u3), (w1, w2, w3)), ((u1, u2, u4), (w1, w2, w4)),
             ((u1, u2, u3), (w1, w2p, w4)), ((u1, u2, u4), (w1, w2p, w3))]
    for n, (us, ws) in enumerate(bases):
        left = frame(*us)
        t = frame(ws[1], ws[0], ws[2])
        right = np.array([t[:, 0], -t[:, 1]])
        for al, be, ga in zip(alpha, beta, gamma):
            a, b = np.zeros((2, 9)), np.zeros((9, 2))
            a[:, 2 * n:2 * n + 2] = inv(left).T @ al
            b[2 * n:2 * n + 2] = be @ inv(right).T
            products.append((a, b, left @ ga @ right))
    for i, u in enumerate((u3, u4)):
        for j, w in enumerate((w2, w2p)):
            a, b = np.zeros((2, 9)), np.zeros((9, 2))
            a[i, 8] = 1.0
            b[8] = inv(np.array([w2, w2p], float))[:, j]
            products.append((a, b, np.outer(u, w)))
    o = np.outer
    patterns = [o(u2, w1), o(u2, w1), o(u3, w1), o(u4, w1),
                o(u1, w2), o(u3, w2), o(u4, w2), np.array([[0, 1], [-1, 0]]),
                o(u1, w2p), o(u3, w2p), o(u4, w2p), np.array([[1, 0], [0, -1]]),
                o(u1, w3), o(u2, w3), o(u1, w4), o(u2, w4)]
    passes = [[] for _ in patterns]
    for a, b, g in products:
        for couple, pattern in zip(passes, patterns):
            s = (g * pattern).sum() / (pattern * pattern).sum()
            if len(couple) < 2 and np.allclose(g, s * pattern):
                lead = b.flat[np.argmax(np.abs(b) > 1e-9)]
                couple.append((np.round(a * s * lead, 12), np.round(b / lead, 12)))
                break
    assert all(len(couple) == 2 for couple in passes)
    return passes


GATE_UP_PASSES = _gate_up_scheme()


def _gate_up_combine(four_passes):
    m = four_passes(0)
    x = m[0] + m[1]
    p = [m[2] - (x + x), m[3] + x]
    m = four_passes(1)
    q = [m[0] + m[1], m[0] + m[2]]
    c = [[(p[i] - q[i]) - q[i], p[i] + q[i]] for i in range(2)]
    c[0][1] += m[3]
    c[1][0] -= m[3]
    m = four_passes(2)
    q = [m[0] + m[1], m[0] + m[2]]
    c = [[c[i][0] + q[i], (c[i][1] - q[i]) - q[i]] for i in range(2)]
    c[0][0] += m[3]
    c[1][1] -= m[3]
    m = four_passes(3)
    return [[c[0][0] + (m[0] - (m[1] + m[1])), c[0][1] + (m[2] - (m[3] + m[3]))],
            [c[1][0] + (m[0] + m[1]), c[1][1] + (m[2] + m[3])]]


def _lincomb(coef, block):
    groups = {}
    for idx in np.argwhere(coef != 0):
        c = float(coef[tuple(idx)])
        v = block(*(int(i) for i in idx))
        if abs(c) in groups:
            g = groups[abs(c)]
            g[1] = g[1] + v if g[0] == c else g[1] - v
        else:
            groups[abs(c)] = [c, v]
    acc = None
    for c, v in groups.values():
        if acc is not None and c == -1.0:
            acc = acc - v
        else:
            v = v if c == 1.0 else v * c
            acc = v if acc is None else acc + v
    return acc


def _strassen_lhs(w):
    f, e = w[0][0] - w[1][1], w[1][0] - w[0][1]
    return [f, f + e, w[0][0] + w[0][1], w[0][1] + w[1][1], w[0][0] - w[0][1], e - f, w[1][1] - w[0][1]]


def _strassen_rhs(x):
    f, e = x[0][1] - x[1][0], x[1][1] - x[0][0]
    return [f, x[0][1] - x[0][0], x[0][0] + x[1][0], f + e, x[0][0] - x[1][0], x[0][0] + x[0][1], f - e]


def _strassen_out(m):
    s = m[2] + m[4]
    d = (m[2] - m[4]) + (m[0] + m[0])
    return [[s, d + (m[3] + m[6])], [d + (m[5] - m[1]), s + (m[5] + m[1]) + (m[3] - m[6])]]


def _dot(a, b):
    return lax.dot_general(a, b, (((1,), (0,)), ((), ())), preferred_element_type=F32)


def _dot_nt(a, b):
    return lax.dot_general(a, b, (((1,), (1,)), ((), ())), preferred_element_type=F32)


def _pack(x):
    return pltpu.bitcast(x.astype(BF16), U32)


def _unpack(x):
    return pltpu.bitcast(x, BF16)


def _vregs(x):
    return [x[i:i + 8] for i in range(0, x.shape[0], 8)]


def _moments(x, progress=None):
    s1 = x - x[0:1]
    s2 = s1 * s1
    if progress is not None:
        s1, s2 = (list(itertools.accumulate(_vregs(z.reshape(-1, 6, 8, T).sum(axis=1).reshape(-1, T))))
                  for z in (s1, s2))
        progress += itertools.chain(*zip(s1, s2))
        s1, s2 = s1[-1], s2[-1]
    mean = jnp.sum(s1, axis=0, keepdims=True) * (1.0 / x.shape[0])
    var = jnp.sum(s2, axis=0, keepdims=True) * (1.0 / x.shape[0]) - mean * mean
    return x[0:1] + mean, lax.rsqrt(jnp.maximum(var, 0.0) + LN_EPS)


class _Order:
    def __init__(self, bits):
        self.bits = pltpu.bitcast(bits, U32) | 1
        self.masks = {}

    def after(self, x, deps):
        if not deps:
            return x
        z = functools.reduce(lax.bitwise_or, [d if d.dtype == U32 else pltpu.bitcast(d, U32) for d in deps])
        if x.shape not in self.masks:
            self.masks[x.shape] = jnp.concatenate([self.bits[:, :x.shape[1]]] * (x.shape[0] // 8), axis=0) != 0
        return lax.select(self.masks[x.shape], x, z if z.shape == x.shape else z[:, :x.shape[1]])

    def after_each(self, x, deps):
        if not any(deps):
            return x
        parts = []
        for busy, run in itertools.groupby(enumerate(deps), key=lambda e: bool(e[1])):
            run = list(run)
            if busy:
                parts += [self.after(x[8 * i:8 * i + 8], d) for i, d in run]
            else:
                parts.append(x[8 * run[0][0]:8 * run[-1][0] + 8])
        return jnp.concatenate(parts, axis=0)


class _Spread:
    def __init__(self, items, count, stop, start=0):
        self.items, self.count, self.slots = iter(items), count, stop - start
        self.now, self.done = -start, 0

    def advance(self, dt):
        self.now += dt
        out = []
        while self.done < min(self.count, self.now * self.count // self.slots):
            self.done += 1
            out.append(next(self.items))
        return out


def _kernel(x_hbm, wq_hbm, wk_hbm, wv_hbm, wo_hbm, wg_hbm, wu_hbm, wd_hbm, c_hbm, wm_hbm,
            out_hbm,
            x_v, wq_v, wk_v, wv_v, wo_v, wg_v, wu_v, wd_v, c_v, wm_v, out_v,
            mod_s, wqkv_s, wo_s, q_s, kvs_s, kb_s, last_s, o_s, x1_s, h2_s, wgu_s, wd_s, act_s, acc_s,
            zero_s, in_sem, out_sem):
    D, S = x_hbm.shape
    F = wg_hbm.shape[1]
    DH = D // N_HEADS
    NB = S // TB
    TPB = TB // T
    NK = S // T
    NU = F // FU
    KS = D // 9
    RB = D // 4
    n_mxu = [T // 16 - n for n in VPU_GROUPS]
    g_off = [2 * sum(VPU_GROUPS[:c]) for c in range(NK + 1)]
    NG = g_off[-1]
    V0 = S // 16
    S0 = V0 + 3 * NK

    def score_at(tile, g):
        return S0 + tile * NG + g

    def mod(i):
        return mod_s[i * D:(i + 1) * D, :]

    def project(w_ref, tiles, *side):
        order = _Order(mod_s[0:8, :])
        nrow = w_ref.shape[0] // 8
        side = [_Spread(items, count, nrow * 5 * TPB) for items, count in side]

        def lhs(lanes, dt):
            deps = [[[y for s in side for y in s.advance(dt)] for _ in lanes] for _ in range(nrow)]
            return [_unpack(order.after_each(w_ref[:, ds], d)) for ds, d in zip(lanes, zip(*deps))]

        main = []
        for z in tiles:
            m = [_dot(w, z[j * T:(j + 1) * T].astype(BF16))
                 for j, w in enumerate(lhs([pl.ds(j * T, T) for j in range(4)], 1))]
            main.append((m[0] + m[1]) + (m[2] + m[3]))
        w, = lhs([pl.ds(4 * T, D - 4 * T)], TPB)
        assert all(s.done == s.count for s in side)
        return [m + _dot(w, z[4 * T:].astype(BF16)) for m, z in zip(main, tiles)]

    copies = {}

    def copy(name, src, dst):
        copies[name] = pltpu.make_async_copy(src, dst, in_sem.at[len(copies)])
        copies[name].start()

    def wait(*names):
        for name in names:
            copies[name].wait()

    copy("c", c_hbm, c_v)
    copy("wm0", wm_hbm.at[:, pl.ds(0, 2 * D)], wm_v.at[:, pl.ds(0, 2 * D)])
    copy("wq", wq_hbm, wq_v)
    copy("wk", wk_hbm, wk_v)
    copy("wv", wv_hbm, wv_v)
    for b in range(NB):
        copy(("x", b), x_hbm.at[:, pl.ds(b * TB, TB)], x_v.at[b])

    def clear(i, carry):
        acc_s[i // 7, pl.ds(i % 7 * 7, 7)] = jnp.zeros((7, RB, T), F32)
        return carry

    zero_s[0] = 0
    lax.fori_loop(0, 7 * NB, clear, 0)

    def modulation(lo, n):
        cf = c_v[...].astype(F32)
        sc = jnp.broadcast_to(cf * jax.nn.sigmoid(cf), (16, D)).astype(BF16)
        row = _dot(sc, wm_v[:, lo:lo + n])[0:1]
        col = lo + lax.broadcasted_iota(jnp.int32, (1, n), 1)
        is_scale = ((col >= D) & (col < 2 * D)) | ((col >= 4 * D) & (col < 5 * D))
        mod_s[lo:lo + n, :] = jnp.broadcast_to(jnp.where(is_scale, 1.0 + row, row), (T, n)).T

    wait("c", "wm0")
    modulation(0, 2 * D)

    wait("wq", "wk", "wv")
    pad = jnp.zeros((24 - DH, D), F32)
    wqkv_s[0:24, :] = _pack(jnp.concatenate([wk_v[...].astype(F32), pad, wv_v[...].astype(F32), pad], axis=0))
    wqkv_s[24:, :] = pltpu.bitcast(wq_v[...].T, U32)
    vpu_keys = []

    def project_qkv(b, *side, then=None):
        h = []
        for t in range(TPB):
            x = x_v[b, :, t * T:(t + 1) * T].astype(F32)
            mean, rstd = _moments(x)
            h.append((x - mean) * rstd * mod(1) + mod(0))
        kvq = project(wqkv_s, h, *side)
        for t, y in enumerate(kvq):
            q_s[b * TPB + t, 0:D, :] = y[48:]
            q_s[b * TPB + t, D:, :] = jnp.zeros((32, T), F32)
        if then is not None:
            then()
        done = []
        for t, y in enumerate(kvq):
            c = b * TPB + t
            k = y[0:24] * (DH ** -0.5 * math.log2(math.e))
            k = jnp.concatenate([k, jnp.zeros((T - 24, T), F32)], axis=0).T
            kvs_s[8 * c:8 * c + 8] = pltpu.bitcast(k.astype(BF16), F32).reshape(8, 8, T)
            is_sum_row = lax.broadcasted_iota(jnp.int32, (24, T), 0) == DH
            kvs_s[V0 + 3 * c:V0 + 3 * c + 3] = jnp.where(is_sum_row, 1.0, y[24:48]).reshape(3, 8, T)
            if VPU_GROUPS[c]:
                vpu_keys.append(k[n_mxu[c] * 16:])
                for d in range(DH):
                    kb = jnp.broadcast_to(vpu_keys[-1][:, d:d + 1], vpu_keys[-1].shape)
                    kb_s[g_off[c]:g_off[c + 1], d] = kb.reshape(-1, 8, T)
                    done += _vregs(kb)
        return done, len(done)

    def copy_the_rest():
        wait(*[("x", b) for b in range(1, NB)])
        copy("wm1", wm_hbm.at[:, pl.ds(2 * D, 4 * D)], wm_v.at[:, pl.ds(2 * D, 4 * D)])
        copy("wo", wo_hbm, wo_v)
        copy("fence", wk_hbm, wk_v)
        for u in range(NU):
            copy(("wg", u), wg_hbm.at[:, pl.ds(u * FU, FU)], wg_v.at[u])
            copy(("wu", u), wu_hbm.at[:, pl.ds(u * FU, FU)], wu_v.at[u])
            copy(("wd", u), wd_hbm.at[:, pl.ds(u * FU, FU)], wd_v.at[u])

    wait(("x", 0))
    work = project_qkv(0, then=copy_the_rest)
    for b in range(1, NB):
        work = project_qkv(b, work)

    for t in range(TPB):
        kvs_s[score_at(t, 0):score_at(t, NG)] = _dot(
            jnp.concatenate(vpu_keys, axis=0)[:, :32].astype(BF16),
            q_s[t, 0:32, :].astype(BF16)).reshape(NG, 8, T)

    def normalize(head, b, acc, safe):
        for t in range(TPB):
            total = jnp.broadcast_to(acc[DH:DH + 1, t * T:(t + 1) * T], (8, T))
            inv = pltpu.reciprocal(total, approx=True)
            inv = inv * (2.0 - total * inv)
            o = [z * inv for z in _vregs(acc[:, t * T:(t + 1) * T])]
            o_s[b * TPB + t, pl.ds(head * DH, 24), :] = jnp.concatenate(o, axis=0)
            probe = (o[0] + o[1]) + (o[2] + total)
            safe = jnp.where((total >= SUM_MIN) & (jnp.abs(probe) <= SUM_MAX), safe, 0.0)
        return safe

    def finish_step(head, v, safe):
        return normalize(head, NB - 1, last_s[0:24] + _dot(v, last_s[24:]), safe)

    def attend_unshifted(step, safe):
        zero = zero_s[0]

        def vpu_scores(head, b):
            for tile in range(b * TPB, (b + 1) * TPB):
                q = q_s[tile, pl.ds(head * DH, 24), :]
                q = [jnp.broadcast_to(q[d:d + 1], (8, T)) for d in range(DH)]
                s = [None, None]
                for d in range(DH):
                    z = kb_s[:, d] * q[d]
                    s[d % 2] = z if d < 2 else s[d % 2] + z
                for g, z in enumerate(_vregs((s[0] + s[1]).reshape(-1, T))):
                    kvs_s[zero + score_at(tile, g)] = z
                    yield

        cols = [(step * HEADS_PER_STEP + n // NB, n % NB) for n in range(HEADS_PER_STEP * NB + 1)]
        side = itertools.chain(*[vpu_scores(*col) for col in cols[1:]])
        cols.pop()
        tiles = [(n, c) for n in range(len(cols)) for c in range(NK)]
        groups = [(n, c, r) for n, c in tiles for r in reversed(range(n_mxu[c]))]
        side = _Spread(side, len(cols) * TPB * NG, 2 * len(groups) + 3 * len(tiles), 1)

        def load(idx, dt):
            side.advance(dt)
            return kvs_s[idx]

        q = [jnp.concatenate([q_s[b * TPB + t, pl.ds(head * DH, 32), :] for t in range(TPB)],
                             axis=1).astype(BF16) for head, b in cols]
        p = {}
        pos = end = 0
        for n, c in [(-1, NK - 1)] + tiles[:-1]:
            rows = []
            if VPU_GROUPS[c]:
                assert side.done >= n * TPB * NG - NG + g_off[c + 1]
                at = [(score_at(cols[n][1] * TPB + t, g_off[c]), score_at(cols[n][1] * TPB + t, g_off[c + 1]))
                      for t in range(TPB)]
                rows = [jnp.exp2(jnp.concatenate([kvs_s[lo:hi].reshape(-1, T) for lo, hi in at], axis=1))]
            end += n_mxu[c] if n >= 0 else 0
            while pos < min(end + AHEAD, len(groups)):
                run = [g for g in groups[pos:end + AHEAD] if g[0] == groups[pos][0]]
                k = jnp.concatenate([load(8 * cc + r, 2) for _, cc, r in run], axis=0)
                e = jnp.exp2(_dot(_unpack(k)[:, :32], q[run[0][0]]))
                p.update((g, e[16 * j:16 * j + 16]) for j, g in enumerate(run))
                pos += len(run)
            v = jnp.concatenate([load(V0 + 3 * c + r, 1) for r in range(3)], axis=0)
            if n < 0:
                safe = finish_step(jnp.maximum(cols[0][0] - 1, 0), v, safe)
                continue
            part = _dot(v, jnp.concatenate([p.pop((n, c, r)) for r in range(n_mxu[c])] + rows, axis=0))
            acc = part if c == 0 else acc + part
            if c == NK - 1:
                safe = normalize(*cols[n], acc, safe)
        last_s[0:24] = acc
        last_s[24:] = jnp.concatenate([p.pop((*tiles[-1], r)) for r in range(T // 16)], axis=0)
        assert side.done == side.count and not p
        return safe

    last_s[...] = jnp.ones(last_s.shape, F32)
    safe = lax.fori_loop(0, N_HEADS // HEADS_PER_STEP, attend_unshifted, jnp.ones((8, T), F32))
    safe = finish_step(N_HEADS - 1, kvs_s[S0 - 3:S0].reshape(24, T), safe)

    @pl.when(jnp.min(safe) < 1.0)
    def _():
        def attend_shifted(i, carry):
            head, tile = i // NK, i % NK
            k = _unpack(kvs_s[0:V0].reshape(S // 2, T))[:, :32]
            v = jnp.concatenate([kvs_s[V0 + 3 * c:V0 + 3 * c + 3].reshape(24, T) for c in range(NK)], axis=1)
            s = _dot(k, q_s[tile, pl.ds(head * DH, 32), :].astype(BF16))
            p = jnp.exp2(s - jnp.max(s, axis=0, keepdims=True))
            acc = _dot(v.astype(BF16), p.astype(BF16))
            o_s[tile, pl.ds(head * DH, 24), :] = acc / acc[DH:DH + 1]
            return carry

        lax.fori_loop(0, N_HEADS * NK, attend_shifted, 0)

    wait("wm1", "wo", *[(name, u) for u in range(NU) for name in ("wg", "wu", "wd")])
    wo_s[...] = pltpu.bitcast(wo_v[...].T, U32)
    modulation(2 * D, 4 * D)
    tile_scale = [math.sqrt(R3 ** ((1 - i) + s)) for i in range(2) for s in range(2)]

    def project_out(b, *side):
        attn = project(wo_s, [o_s[b * TPB + t, 0:D, :] for t in range(TPB)], *side)
        for t in range(TPB):
            x1_s[b, t] = x_v[b, :, t * T:(t + 1) * T].astype(F32) + mod(2) * attn[t]
        progress = []
        moments = [_moments(x1_s[b, t], progress) for t in range(TPB)]

        def operands(start):
            h2 = []
            for t, (mean, rstd) in enumerate(moments):
                mean = pltpu.bitcast(jnp.broadcast_to(mean, (8, T)), U32)
                mean = pltpu.bitcast(_Order(mod_s[0:8, :]).after(mean, [start()]), F32)[0:1]
                z = (x1_s[b, t] - mean) * (rstd * tile_scale[t]) * mod(4)
                h2.append(z + (mod(3) if tile_scale[t] == 1.0 else mod(3) * tile_scale[t]))
            for s in range(2):
                for r, couple in enumerate(GATE_UP_PASSES):
                    z = [_lincomb(a, lambda i, k: h2[2 * i + s][k * KS:(k + 1) * KS]) for a, _ in couple]
                    z = pltpu.bitcast(jnp.concatenate(z, axis=0).astype(BF16).T, U32)
                    h2_s[b, r, s * T // 2:(s + 1) * T // 2, :] = z
                    yield from (z[i:i + 8] for i in range(8, T // 2, 16))

        return (progress, len(progress)), lambda start: (operands(start), 2 * 16 * T // 32)

    def prepare_gate_up(u, t):
        terms = sorted(((int(np.argwhere(coef != 0)[0, 0]) // 2, r, m, coef)
                        for r, couple in enumerate(GATE_UP_PASSES) for m, (_, coef) in enumerate(couple)),
                       key=lambda e: e[:3])

        def work():
            for n, w_v in enumerate((wg_v, wu_v)):
                w = [w_v[u, :, pl.ds((2 * j + t) * T, T)].astype(F32) for j in range(2)]
                done = [_pack(_lincomb(coef, lambda k, j: w[j][k * KS:(k + 1) * KS])) for *_, coef in terms]
                for i in range(KS // 16):
                    for (_, r, m, _), y in zip(terms, done):
                        y = y[8 * i:8 * i + 8]
                        wgu_s[2 * t + n, r, pl.ds(m * KS // 2 + 8 * i, 8), :] = y
                        yield y

        return work(), 2 * 16 * T // 16

    def prepare_down(u):
        def work():
            def block(r1, r2, j, t):
                w = wd_v[u, pl.ds((2 * r1 + r2) * RB, RB), pl.ds((2 * j + t) * T, T)].astype(F32)
                return w if r1 + r2 == j + t else w * R3 ** (r1 + r2 - j - t)

            outer = [[_strassen_lhs([[block(r1, r2, j, t) for j in range(2)] for r1 in range(2)])
                      for t in range(2)] for r2 in range(2)]
            done = [_pack(y) for r in range(7)
                    for y in _strassen_lhs([[outer[r2][t][r] for t in range(2)] for r2 in range(2)])]
            for r, y in enumerate(done):
                wd_s[r] = y
            outer = [pltpu.bitcast(z, U32) for row in outer for forms in row for z in forms]
            for i in range(RB // 16):
                yield from (z[16 * i + k:16 * i + k + 8] for z in outer for k in (0, 8))
                yield from (y[8 * i:8 * i + 8] for y in done)

        return work(), (56 + 49) * RB // 16

    def finish(b, inner):
        def work():
            for r2 in range(2):
                for s in range(2):
                    y = _strassen_out([inner[r][r2][s] for r in range(7)])
                    done = []
                    for r1 in range(2):
                        for i in range(2):
                            rows = pl.ds((2 * r1 + r2) * RB, RB)
                            tile = 2 * (1 - i) + s
                            gate = mod_s[pl.ds(5 * D + (2 * r1 + r2) * RB, RB), :]
                            z = x1_s[b, tile, rows, :] + gate * (0.125 * R3 ** -(r1 + r2 + i + s)) * y[r1][i]
                            out_v[b, rows, pl.ds(tile * T, T)] = z.astype(out_v.dtype)
                            done.append(_vregs(z))
                    yield from itertools.chain(*zip(*done))

        return work(), TPB * D // 8

    slabs = TB // (2 * MH)

    class Ffn:
        def __init__(self):
            self.order = _Order(mod_s[0:8, :])
            self.side = []
            self.due = []

        def run_under(self, work, stop, start=0):
            items, count = work
            slots = 2 * 16 * slabs
            items = itertools.chain(items, itertools.repeat(self.order.bits))
            self.side.append(_Spread(zip(*[items] * (MH // 16)), -(-count // (MH // 16)),
                                     int(stop * slots), int(start * slots)))

        def drained(self):
            return all(s.done == s.count for s in self.side)

        def lhs(self, x, due, side):
            due = [pltpu.bitcast(z, U32).reshape(-1, 16, T) for z in due]
            due = [z[:, k:k + 8].reshape(x.shape) for z in due for k in (0, 8)]
            for s in side:
                due += [jnp.concatenate(z, axis=0) for z in s.advance(1)]
            return _unpack(self.order.after(x, due))

        def next_round(self, rows):
            self.due = [(n - 1, z) for n, z in self.due]
            now = [z for n, z in self.due if n < 0 and z.shape[0] == rows]
            self.due = [(n, z) for n, z in self.due if n >= 0 or z.shape[0] != rows]
            return now

        def product(self, b, n, slab):
            def four_passes(k):
                due = self.next_round(MH)
                rows = pl.ds(slab * MH // 2, MH // 2)
                return [_dot(self.lhs(h2_s[b, 4 * k + r, rows, :], due[r::4], self.side),
                             _unpack(wgu_s[n, 4 * k + r])) for r in range(4)]

            return _gate_up_combine(four_passes)

        def gate_up(self, b, t, midway, at):
            parts = []
            for slab in range(slabs):
                g = self.product(b, 2 * t, slab)

                def silu2(i, j):
                    th = jnp.tanh(g[i][j] * (0.5 / tile_scale[2 * i + slab * MH // T]))
                    z = g[i][j] if j + t == 0 else g[i][j] * R3 ** (j + t)
                    return z + z * th

                act = [[silu2(i, j) for j in range(2)] for i in range(2)]
                self.due += [(3, z) for z in act[0] + act[1]]
                up = self.product(b, 2 * t + 1, slab)
                parts.append(_strassen_rhs([[act[1 - i][j] * up[1 - i][j] for i in range(2)] for j in range(2)]))
                self.due += [(3, z) for z in parts[-1]]
                if midway is not None and slab == at:
                    midway()
            return [jnp.concatenate(z, axis=0) for z in zip(*parts)]

        def first_half(self, b, midway=None):
            for r, z in enumerate(self.gate_up(b, 0, midway, 2)):
                act_s[b, r] = z

        def second_half(self, b, midway, at=2, last=False):
            outer = [[act_s[b, r] for r in range(7)], self.gate_up(b, 1, midway, at)]

            def down():
                rhs = [y for r in range(7)
                       for y in _strassen_rhs([[outer[t][r][:T], outer[t][r][T:]] for t in range(2)])]
                inner, m = [], {}
                for n, r in enumerate(7 * g + k for g in range(7) for k in (2, 4, 0, 3, 6, 1, 5)):
                    if n % 4 == 0:
                        due = self.next_round(RB)
                    y = acc_s[b, r] + _dot_nt(self.lhs(wd_s[r], due[n % 4::4], []), rhs[r].astype(BF16))
                    if not last:
                        acc_s[b, r] = y
                        continue
                    m[r % 7] = y
                    if n % 7 == 6:
                        inner.append(_strassen_out(m))
                        self.due += [(1, z) for z in inner[-1][0] + inner[-1][1]]
                if last:
                    self.due = [(n, z) for n, z in self.due if z.shape[0] != RB]
                    self.run_under(finish(b, inner), 0.9 if b < NB - 2 else 0.75, 0.05)

            return down

    norm0, operands0 = project_out(0, prepare_gate_up(0, 0))
    norm1, operands1 = project_out(1, norm0, prepare_gate_up(0, 1))
    norm2, operands2 = project_out(2, norm1, operands0(lambda: x1_s[1, 0, 0:8]))
    norm3, operands3 = project_out(3, norm2, operands1(lambda: x1_s[2, 0, 0:8]))
    ffn = Ffn()
    ffn.run_under(norm3, 2, 0.5)
    ffn.run_under(operands2(lambda: x1_s[3, 0, 0:8]), 2)
    ffn.run_under(operands3(lambda: act_s[0, 0, TB // 2 - 8:]), 3, 2)
    for b in range(NB):
        ffn.first_half(b)

    def unit(u, carry):
        ffn = Ffn()
        ffn.run_under(prepare_down(u), 2.75)
        ffn.run_under(prepare_gate_up(u + 1, 0), NB, 2.9)
        downs = [None, None]
        for b in range(NB):
            downs.append(ffn.second_half(b, downs.pop(0)))
        assert ffn.drained()
        ffn.run_under(prepare_gate_up(u + 1, 1), NB, 1.75)
        for b in range(NB):
            ffn.first_half(b, downs.pop(0) if downs else None)
        assert ffn.drained()
        return carry

    lax.fori_loop(0, NU - 1, unit, 0)

    def out_copy(b):
        return pltpu.make_async_copy(out_v.at[b], out_hbm.at[:, pl.ds(b * TB, TB)], out_sem.at[b])

    ffn = Ffn()
    ffn.run_under(prepare_down(NU - 1), 1.75)
    down = None
    for b in range(NB):
        down = ffn.second_half(b, down, at=NB - 1 - b, last=True)
    assert ffn.drained()
    for b in range(NB - 1):
        out_copy(b).start()
    wait("fence")
    down()
    ffn.side[-1].advance(2 * ffn.side[-1].slots)
    assert ffn.drained()
    out_copy(NB - 1).start()
    for b in range(NB):
        out_copy(b).wait()


@jax.jit
def pallas_adaLN_cond__grouped_kv_mqa__swiglu_ffn__prompt_kernel(
    A_x: jax.Array,
    A_wq: jax.Array,
    A_wk: jax.Array,
    A_wv: jax.Array,
    A_wo: jax.Array,
    B_x: jax.Array,
    B_w_gate: jax.Array,
    B_w_up: jax.Array,
    B_w_down: jax.Array,
    c: jax.Array,
    w_mod: jax.Array,
):
    del B_x
    B, S, D = A_x.shape
    F = B_w_gate.shape[1]
    assert (B, S, D) == (1, T * len(VPU_GROUPS), 576) and F % FU == 0 and A_x.dtype == BF16
    DH = D // N_HEADS
    NB, NU, NK = S // TB, F // FU, S // T
    NG = 2 * sum(VPU_GROUPS)
    vmem = pltpu.VMEM
    scratch = [
        vmem((NB, D, TB), BF16),
        vmem((D, D), BF16),
        vmem((DH, D), BF16),
        vmem((DH, D), BF16),
        vmem((D, D), BF16),
        vmem((NU, D, FU), BF16),
        vmem((NU, D, FU), BF16),
        vmem((NU, D, FU), BF16),
        vmem((1, D), BF16),
        vmem((D, 6 * D), BF16),
        vmem((NB, D, TB), BF16),
        vmem((6 * D, T), F32),
        vmem(((D + 48) // 2, D), U32),
        vmem((D // 2, D), U32),
        vmem((NK, D + 32, T), F32),
        vmem((S // 16 + 3 * NK + NK * NG, 8, T), F32),
        vmem((NG, DH, 8, T), F32),
        vmem((24 + T, TB), F32),
        vmem((NK, D + 8, T), F32),
        vmem((NB, TB // T, D, T), F32),
        vmem((NB, 16, TB // 4, T), U32),
        vmem((4, 16, T // 2, T), U32),
        vmem((49, D // 8, T), U32),
        vmem((NB, 7, TB // 2, T), F32),
        vmem((NB, 49, D // 4, T), F32),
        pltpu.SMEM((1,), jnp.int32),
        pltpu.SemaphoreType.DMA((8 + NB + 3 * NU,)),
        pltpu.SemaphoreType.DMA((NB,)),
    ]
    out = pl.pallas_call(
        _kernel,
        out_shape=jax.ShapeDtypeStruct((D, S), BF16),
        in_specs=[pl.BlockSpec(memory_space=pl.ANY)] * 10,
        out_specs=pl.BlockSpec(memory_space=pl.ANY),
        scratch_shapes=scratch,
        compiler_params=pltpu.CompilerParams(vmem_limit_bytes=110 * 1024 * 1024),
        name="adaln_mqa_swiglu",
    )(A_x.reshape(S, D).T, A_wq, A_wk.T, A_wv.T, A_wo, B_w_gate, B_w_up, B_w_down.T, c, w_mod)
    return out.T.reshape(B, S, D)
```

```python
import functools
import itertools
import math

import jax
import jax.numpy as jnp
import numpy as np
from jax import lax
import jax.experimental.pallas as pl
import jax.experimental.pallas.tpu as pltpu

F32 = jnp.float32
BF16 = jnp.bfloat16
U32 = jnp.uint32

N_HEADS = 32
LN_EPS = 1e-5
T = 128
TB = 512
FU = 512
MH = 64
VPU_GROUPS = (1, 2, 1, 2, 2, 1, 2, 2, 1, 2, 2, 1, 2, 1, 1, 0)
AHEAD = 8
HEADS_PER_STEP = 2
SUM_MIN = 2.0 ** -30
SUM_MAX = 2.0 ** 120
R3 = math.sqrt(3.0)


def _gate_up_scheme():
    e = [[np.outer(np.eye(2)[i], np.eye(2)[j]) for j in range(2)] for i in range(2)]
    alpha = [e[0][0] + e[1][1], e[1][0] + e[1][1], e[0][0], e[1][1],
             e[0][0] + e[0][1], e[1][0] - e[0][0], e[0][1] - e[1][1]]
    beta = [e[0][0] + e[1][1], e[0][0], e[0][1] - e[1][1], e[1][0] - e[0][0],
            e[1][1], e[0][0] + e[0][1], e[1][0] + e[1][1]]
    gamma = [e[0][0] + e[1][1], e[1][0] - e[1][1], e[0][1] + e[1][1], e[0][0] + e[1][0],
             e[0][1] - e[0][0], e[1][1], e[0][0]]

    def inv(m):
        det = m[0, 0] * m[1, 1] - m[0, 1] * m[1, 0]
        return np.array([[m[1, 1], -m[0, 1]], [-m[1, 0], m[0, 0]]]) / det

    def frame(p1, p2, p3):
        m = np.array([p1, p2], float).T
        return m * (inv(m) @ np.array(p3, float))

    u1, u2, u3, u4 = (1, 1), (-2, 1), (1, 0), (0, 1)
    w1, w2, w2p, w3, w4 = (1, 1), (-2, 1), (1, -2), (1, 0), (0, 1)
    products = []
    bases = [((u1, u2, u3), (w1, w2, w3)), ((u1, u2, u4), (w1, w2, w4)),
             ((u1, u2, u3), (w1, w2p, w4)), ((u1, u2, u4), (w1, w2p, w3))]
    for n, (us, ws) in enumerate(bases):
        left = frame(*us)
        t = frame(ws[1], ws[0], ws[2])
        right = np.array([t[:, 0], -t[:, 1]])
        for al, be, ga in zip(alpha, beta, gamma):
            a, b = np.zeros((2, 9)), np.zeros((9, 2))
            a[:, 2 * n:2 * n + 2] = inv(left).T @ al
            b[2 * n:2 * n + 2] = be @ inv(right).T
            products.append((a, b, left @ ga @ right))
    for i, u in enumerate((u3, u4)):
        for j, w in enumerate((w2, w2p)):
            a, b = np.zeros((2, 9)), np.zeros((9, 2))
            a[i, 8] = 1.0
            b[8] = inv(np.array([w2, w2p], float))[:, j]
            products.append((a, b, np.outer(u, w)))
    o = np.outer
    patterns = [o(u2, w1), o(u2, w1), o(u3, w1), o(u4, w1),
                o(u1, w2), o(u3, w2), o(u4, w2), np.array([[0, 1], [-1, 0]]),
                o(u1, w2p), o(u3, w2p), o(u4, w2p), np.array([[1, 0], [0, -1]]),
                o(u1, w3), o(u2, w3), o(u1, w4), o(u2, w4)]
    passes = [[] for _ in patterns]
    for a, b, g in products:
        for couple, pattern in zip(passes, patterns):
            s = (g * pattern).sum() / (pattern * pattern).sum()
            if len(couple) < 2 and np.allclose(g, s * pattern):
                lead = b.flat[np.argmax(np.abs(b) > 1e-9)]
                couple.append((np.round(a * s * lead, 12), np.round(b / lead, 12)))
                break
    assert all(len(couple) == 2 for couple in passes)
    return passes


GATE_UP_PASSES = _gate_up_scheme()


def _gate_up_combine(four_passes):
    m = four_passes(0)
    x = m[0] + m[1]
    p = [m[2] - (x + x), m[3] + x]
    m = four_passes(1)
    q = [m[0] + m[1], m[0] + m[2]]
    c = [[(p[i] - q[i]) - q[i], p[i] + q[i]] for i in range(2)]
    c[0][1] += m[3]
    c[1][0] -= m[3]
    m = four_passes(2)
    q = [m[0] + m[1], m[0] + m[2]]
    c = [[c[i][0] + q[i], (c[i][1] - q[i]) - q[i]] for i in range(2)]
    c[0][0] += m[3]
    c[1][1] -= m[3]
    m = four_passes(3)
    return [[c[0][0] + (m[0] - (m[1] + m[1])), c[0][1] + (m[2] - (m[3] + m[3]))],
            [c[1][0] + (m[0] + m[1]), c[1][1] + (m[2] + m[3])]]


def _lincomb(coef, block):
    groups = {}
    for idx in np.argwhere(coef != 0):
        c = float(coef[tuple(idx)])
        v = block(*(int(i) for i in idx))
        if abs(c) in groups:
            g = groups[abs(c)]
            g[1] = g[1] + v if g[0] == c else g[1] - v
        else:
            groups[abs(c)] = [c, v]
    acc = None
    for c, v in groups.values():
        if acc is not None and c == -1.0:
            acc = acc - v
        else:
            v = v if c == 1.0 else v * c
            acc = v if acc is None else acc + v
    return acc


def _strassen_lhs(w):
    f, e = w[0][0] - w[1][1], w[1][0] - w[0][1]
    return [f, f + e, w[0][0] + w[0][1], w[0][1] + w[1][1], w[0][0] - w[0][1], e - f, w[1][1] - w[0][1]]


def _strassen_rhs(x):
    f, e = x[0][1] - x[1][0], x[1][1] - x[0][0]
    return [f, x[0][1] - x[0][0], x[0][0] + x[1][0], f + e, x[0][0] - x[1][0], x[0][0] + x[0][1], f - e]


def _strassen_out(m):
    s = m[2] + m[4]
    d = (m[2] - m[4]) + (m[0] + m[0])
    return [[s, d + (m[3] + m[6])], [d + (m[5] - m[1]), s + (m[5] + m[1]) + (m[3] - m[6])]]


def _dot(a, b):
    return lax.dot_general(a, b, (((1,), (0,)), ((), ())), preferred_element_type=F32)


def _dot_nt(a, b):
    return lax.dot_general(a, b, (((1,), (1,)), ((), ())), preferred_element_type=F32)


def _pack(x):
    return pltpu.bitcast(x.astype(BF16), U32)


def _unpack(x):
    return pltpu.bitcast(x, BF16)


def _vregs(x):
    return [x[i:i + 8] for i in range(0, x.shape[0], 8)]


def _moments(x, progress=None):
    s1 = x - x[0:1]
    s2 = s1 * s1
    if progress is not None:
        s1, s2 = (list(itertools.accumulate(_vregs(z.reshape(-1, 6, 8, T).sum(axis=1).reshape(-1, T))))
                  for z in (s1, s2))
        progress += itertools.chain(*zip(s1, s2))
        s1, s2 = s1[-1], s2[-1]
    mean = jnp.sum(s1, axis=0, keepdims=True) * (1.0 / x.shape[0])
    var = jnp.sum(s2, axis=0, keepdims=True) * (1.0 / x.shape[0]) - mean * mean
    return x[0:1] + mean, lax.rsqrt(jnp.maximum(var, 0.0) + LN_EPS)


class _Order:
    def __init__(self, bits):
        self.bits = pltpu.bitcast(bits, U32) | 1
        self.masks = {}

    def after(self, x, deps):
        if not deps:
            return x
        z = functools.reduce(lax.bitwise_or, [d if d.dtype == U32 else pltpu.bitcast(d, U32) for d in deps])
        if x.shape not in self.masks:
            self.masks[x.shape] = jnp.concatenate([self.bits[:, :x.shape[1]]] * (x.shape[0] // 8), axis=0) != 0
        return lax.select(self.masks[x.shape], x, z if z.shape == x.shape else z[:, :x.shape[1]])

    def after_each(self, x, deps):
        if not any(deps):
            return x
        parts = []
        for busy, run in itertools.groupby(enumerate(deps), key=lambda e: bool(e[1])):
            run = list(run)
            if busy:
                parts += [self.after(x[8 * i:8 * i + 8], d) for i, d in run]
            else:
                parts.append(x[8 * run[0][0]:8 * run[-1][0] + 8])
        return jnp.concatenate(parts, axis=0)


class _Spread:
    def __init__(self, items, count, stop, start=0):
        self.items, self.count, self.slots = iter(items), count, stop - start
        self.now, self.done = -start, 0

    def advance(self, dt):
        self.now += dt
        out = []
        while self.done < min(self.count, self.now * self.count // self.slots):
            self.done += 1
            out.append(next(self.items))
        return out


def _kernel(x_hbm, wq_hbm, wk_hbm, wv_hbm, wo_hbm, wg_hbm, wu_hbm, wd_hbm, c_hbm, wm_hbm,
            out_hbm,
            x_v, wq_v, wk_v, wv_v, wo_v, wg_v, wu_v, wd_v, c_v, wm_v, out_v,
            mod_s, wqkv_s, wo_s, q_s, kvs_s, kb_s, last_s, o_s, x1_s, h2_s, wgu_s, wd_s, act_s, acc_s,
            zero_s, in_sem, w_sem, out_sem):
    D, S = x_hbm.shape
    F = wg_hbm.shape[1]
    DH = D // N_HEADS
    NB = S // TB
    TPB = TB // T
    NK = S // T
    NU = F // FU
    KS = D // 9
    RB = D // 4
    n_mxu = [T // 16 - n for n in VPU_GROUPS]
    g_off = [2 * sum(VPU_GROUPS[:c]) for c in range(NK + 1)]
    NG = g_off[-1]
    V0 = S // 16
    S0 = V0 + 3 * NK

    def score_at(tile, g):
        return S0 + tile * NG + g

    def mod(i):
        return mod_s[i * D:(i + 1) * D, :]

    def project(w_ref, tiles, *side):
        order = _Order(mod_s[0:8, :])
        nrow = w_ref.shape[0] // 8
        side = [_Spread(items, count, nrow * 5 * TPB) for items, count in side]

        def lhs(lanes, dt):
            deps = [[[y for s in side for y in s.advance(dt)] for _ in lanes] for _ in range(nrow)]
            return [_unpack(order.after_each(w_ref[:, ds], d)) for ds, d in zip(lanes, zip(*deps))]

        main = []
        for z in tiles:
            m = [_dot(w, z[j * T:(j + 1) * T].astype(BF16))
                 for j, w in enumerate(lhs([pl.ds(j * T, T) for j in range(4)], 1))]
            main.append((m[0] + m[1]) + (m[2] + m[3]))
        w, = lhs([pl.ds(4 * T, D - 4 * T)], TPB)
        assert all(s.done == s.count for s in side)
        return [m + _dot(w, z[4 * T:].astype(BF16)) for m, z in zip(main, tiles)]

    copies = {}

    def copy(name, src, dst):
        copies[name] = pltpu.make_async_copy(src, dst, in_sem.at[len(copies)])
        copies[name].start()

    def wait(*names):
        for name in names:
            copies[name].wait()

    copy("c", c_hbm, c_v)
    copy("wm0", wm_hbm.at[:, pl.ds(0, 2 * D)], wm_v.at[:, pl.ds(0, 2 * D)])
    copy("wq", wq_hbm, wq_v)
    copy("wk", wk_hbm, wk_v)
    copy("wv", wv_hbm, wv_v)
    for b in range(NB):
        copy(("x", b), x_hbm.at[:, pl.ds(b * TB, TB)], x_v.at[b])

    def clear(i, carry):
        acc_s[i // 7, pl.ds(i % 7 * 7, 7)] = jnp.zeros((7, RB, T), F32)
        return carry

    zero_s[0] = 0
    lax.fori_loop(0, 7 * NB, clear, 0)

    def modulation(lo, n):
        cf = c_v[...].astype(F32)
        sc = jnp.broadcast_to(cf * jax.nn.sigmoid(cf), (16, D)).astype(BF16)
        row = _dot(sc, wm_v[:, lo:lo + n])[0:1]
        col = lo + lax.broadcasted_iota(jnp.int32, (1, n), 1)
        is_scale = ((col >= D) & (col < 2 * D)) | ((col >= 4 * D) & (col < 5 * D))
        mod_s[lo:lo + n, :] = jnp.broadcast_to(jnp.where(is_scale, 1.0 + row, row), (T, n)).T

    wait("c", "wm0")
    modulation(0, 2 * D)

    wait("wq", "wk", "wv")
    pad = jnp.zeros((24 - DH, D), F32)
    wqkv_s[0:24, :] = _pack(jnp.concatenate([wk_v[...].astype(F32), pad, wv_v[...].astype(F32), pad], axis=0))
    wqkv_s[24:, :] = pltpu.bitcast(wq_v[...].T, U32)
    vpu_keys = []

    def project_qkv(b, *side, then=None):
        h = []
        for t in range(TPB):
            x = x_v[b, :, t * T:(t + 1) * T].astype(F32)
            mean, rstd = _moments(x)
            h.append((x - mean) * rstd * mod(1) + mod(0))
        kvq = project(wqkv_s, h, *side)
        for t, y in enumerate(kvq):
            q = jnp.concatenate([y[48:], jnp.zeros((24, T), F32)], axis=0)
            for head in range(N_HEADS + 1):
                q_s[b * TPB + t, head] = q[head * DH:head * DH + 24]
        if then is not None:
            then()
        done = []
        for t, y in enumerate(kvq):
            c = b * TPB + t
            k = y[0:24] * (DH ** -0.5 * math.log2(math.e))
            k = jnp.concatenate([k, jnp.zeros((T - 24, T), F32)], axis=0).T
            kvs_s[8 * c:8 * c + 8] = pltpu.bitcast(k.astype(BF16), F32).reshape(8, 8, T)
            is_sum_row = lax.broadcasted_iota(jnp.int32, (24, T), 0) == DH
            kvs_s[V0 + 3 * c:V0 + 3 * c + 3] = jnp.where(is_sum_row, 1.0, y[24:48]).reshape(3, 8, T)
            if VPU_GROUPS[c]:
                vpu_keys.append(k[n_mxu[c] * 16:])
                for d in range(DH):
                    kb = jnp.broadcast_to(vpu_keys[-1][:, d:d + 1], vpu_keys[-1].shape)
                    kb_s[g_off[c]:g_off[c + 1], d] = kb.reshape(-1, 8, T)
                    done += _vregs(kb)
        return done, len(done)

    def fetch(n, u):
        cols = pl.ds(u * FU if isinstance(u, int) else pl.multiple_of(u * FU, FU), FU)
        return pltpu.make_async_copy((wg_hbm, wu_hbm, wd_hbm)[n].at[:, cols], (wg_v, wu_v, wd_v)[n], w_sem.at[n])

    def copy_the_rest():
        wait(*[("x", b) for b in range(1, NB)])
        copy("wm1", wm_hbm.at[:, pl.ds(2 * D, 4 * D)], wm_v.at[:, pl.ds(2 * D, 4 * D)])
        copy("wo", wo_hbm, wo_v)
        for n in range(3):
            fetch(n, 0).start()

    wait(("x", 0))
    work = project_qkv(0, then=copy_the_rest)
    for b in range(1, NB):
        work = project_qkv(b, work)

    def queries(tile, head):
        return jnp.concatenate([q_s[tile, head], jnp.zeros((8, T), F32)], axis=0)

    for t in range(TPB):
        kvs_s[score_at(t, 0):score_at(t, NG)] = _dot(
            jnp.concatenate(vpu_keys, axis=0)[:, :32].astype(BF16),
            queries(t, 0).astype(BF16)).reshape(NG, 8, T)

    def normalize(head, b, acc, safe):
        for t in range(TPB):
            total = jnp.broadcast_to(acc[DH:DH + 1, t * T:(t + 1) * T], (8, T))
            inv = pltpu.reciprocal(total, approx=True)
            inv = inv * (2.0 - total * inv)
            o = [z * inv for z in _vregs(acc[:, t * T:(t + 1) * T])]
            o_s[b * TPB + t, pl.ds(head * DH, 24), :] = jnp.concatenate(o, axis=0)
            probe = (o[0] + o[1]) + (o[2] + total)
            safe = jnp.where((total >= SUM_MIN) & (jnp.abs(probe) <= SUM_MAX), safe, 0.0)
        return safe

    def finish_step(head, v, safe):
        return normalize(head, NB - 1, last_s[0:24] + _dot(v, last_s[24:]), safe)

    def attend_unshifted(step, safe):
        zero = zero_s[0]

        def vpu_scores(head, b):
            for tile in range(b * TPB, (b + 1) * TPB):
                q = q_s[tile, head]
                q = [jnp.broadcast_to(q[d:d + 1], (8, T)) for d in range(DH)]
                s = [None, None]
                for d in range(DH):
                    z = kb_s[:, d] * q[d]
                    s[d % 2] = z if d < 2 else s[d % 2] + z
                for g, z in enumerate(_vregs((s[0] + s[1]).reshape(-1, T))):
                    kvs_s[zero + score_at(tile, g)] = z
                    yield

        cols = [(step * HEADS_PER_STEP + n // NB, n % NB) for n in range(HEADS_PER_STEP * NB + 1)]
        side = itertools.chain(*[vpu_scores(*col) for col in cols[1:]])
        cols.pop()
        tiles = [(n, c) for n in range(len(cols)) for c in range(NK)]
        groups = [(n, c, r) for n, c in tiles for r in reversed(range(n_mxu[c]))]
        side = _Spread(side, len(cols) * TPB * NG, 2 * len(groups) + 3 * len(tiles), 1)

        def load(idx, dt):
            side.advance(dt)
            return kvs_s[idx]

        q = [jnp.concatenate([queries(b * TPB + t, head) for t in range(TPB)],
                             axis=1).astype(BF16) for head, b in cols]
        p = {}
        pos = end = 0
        for n, c in [(-1, NK - 1)] + tiles[:-1]:
            rows = []
            if VPU_GROUPS[c]:
                assert side.done >= n * TPB * NG - NG + g_off[c + 1]
                at = [(score_at(cols[n][1] * TPB + t, g_off[c]), score_at(cols[n][1] * TPB + t, g_off[c + 1]))
                      for t in range(TPB)]
                rows = [jnp.exp2(jnp.concatenate([kvs_s[lo:hi].reshape(-1, T) for lo, hi in at], axis=1))]
            end += n_mxu[c] if n >= 0 else 0
            while pos < min(end + AHEAD, len(groups)):
                run = [g for g in groups[pos:end + AHEAD] if g[0] == groups[pos][0]]
                k = jnp.concatenate([load(8 * cc + r, 2) for _, cc, r in run], axis=0)
                e = jnp.exp2(_dot(_unpack(k)[:, :32], q[run[0][0]]))
                p.update((g, e[16 * j:16 * j + 16]) for j, g in enumerate(run))
                pos += len(run)
            v = jnp.concatenate([load(V0 + 3 * c + r, 1) for r in range(3)], axis=0)
            if n < 0:
                safe = finish_step(jnp.maximum(cols[0][0] - 1, 0), v, safe)
                continue
            part = _dot(v, jnp.concatenate([p.pop((n, c, r)) for r in range(n_mxu[c])] + rows, axis=0))
            acc = part if c == 0 else acc + part
            if c == NK - 1:
                safe = normalize(*cols[n], acc, safe)
        last_s[0:24] = acc
        last_s[24:] = jnp.concatenate([p.pop((*tiles[-1], r)) for r in range(T // 16)], axis=0)
        assert side.done == side.count and not p
        return safe

    last_s[...] = jnp.ones(last_s.shape, F32)
    safe = lax.fori_loop(0, N_HEADS // HEADS_PER_STEP, attend_unshifted, jnp.ones((8, T), F32))
    safe = finish_step(N_HEADS - 1, kvs_s[S0 - 3:S0].reshape(24, T), safe)

    @pl.when(jnp.min(safe) < 1.0)
    def _():
        def attend_shifted(i, carry):
            head, tile = i // NK, i % NK
            k = _unpack(kvs_s[0:V0].reshape(S // 2, T))[:, :32]
            v = jnp.concatenate([kvs_s[V0 + 3 * c:V0 + 3 * c + 3].reshape(24, T) for c in range(NK)], axis=1)
            s = _dot(k, queries(tile, head).astype(BF16))
            p = jnp.exp2(s - jnp.max(s, axis=0, keepdims=True))
            acc = _dot(v.astype(BF16), p.astype(BF16))
            o_s[tile, pl.ds(head * DH, 24), :] = acc / acc[DH:DH + 1]
            return carry

        lax.fori_loop(0, N_HEADS * NK, attend_shifted, 0)

    wait("wm1", "wo")
    fetch(0, 0).wait()
    fetch(1, 0).wait()
    wo_s[...] = pltpu.bitcast(wo_v[...].T, U32)
    modulation(2 * D, 4 * D)
    tile_scale = [math.sqrt(R3 ** ((1 - i) + s)) for i in range(2) for s in range(2)]

    def project_out(b, *side):
        attn = project(wo_s, [o_s[b * TPB + t, 0:D, :] for t in range(TPB)], *side)
        for t in range(TPB):
            x1_s[b, t] = x_v[b, :, t * T:(t + 1) * T].astype(F32) + mod(2) * attn[t]
        progress = []
        moments = [_moments(x1_s[b, t], progress) for t in range(TPB)]

        def operands(start):
            h2 = []
            for t, (mean, rstd) in enumerate(moments):
                mean = pltpu.bitcast(jnp.broadcast_to(mean, (8, T)), U32)
                mean = pltpu.bitcast(_Order(mod_s[0:8, :]).after(mean, [start()]), F32)[0:1]
                z = (x1_s[b, t] - mean) * (rstd * tile_scale[t]) * mod(4)
                h2.append(z + (mod(3) if tile_scale[t] == 1.0 else mod(3) * tile_scale[t]))
            for s in range(2):
                for r, couple in enumerate(GATE_UP_PASSES):
                    z = [_lincomb(a, lambda i, k: h2[2 * i + s][k * KS:(k + 1) * KS]) for a, _ in couple]
                    z = pltpu.bitcast(jnp.concatenate(z, axis=0).astype(BF16).T, U32)
                    h2_s[b, r, s * T // 2:(s + 1) * T // 2, :] = z
                    yield from (z[i:i + 8] for i in range(8, T // 2, 16))

        return (progress, len(progress)), lambda start: (operands(start), 2 * 16 * T // 32)

    def prepare_gate_up(t):
        terms = sorted(((int(np.argwhere(coef != 0)[0, 0]) // 2, r, m, coef)
                        for r, couple in enumerate(GATE_UP_PASSES) for m, (_, coef) in enumerate(couple)),
                       key=lambda e: e[:3])

        def work():
            for n, w_v in enumerate((wg_v, wu_v)):
                w = [w_v[:, pl.ds((2 * j + t) * T, T)].astype(F32) for j in range(2)]
                done = [_pack(_lincomb(coef, lambda k, j: w[j][k * KS:(k + 1) * KS])) for *_, coef in terms]
                for i in range(KS // 16):
                    for (_, r, m, _), y in zip(terms, done):
                        y = y[8 * i:8 * i + 8]
                        wgu_s[2 * t + n, r, pl.ds(m * KS // 2 + 8 * i, 8), :] = y
                        yield y

        return work(), 2 * 16 * T // 16

    def prepare_down():
        def work():
            def block(r1, r2, j, t):
                w = wd_v[pl.ds((2 * r1 + r2) * RB, RB), pl.ds((2 * j + t) * T, T)].astype(F32)
                return w if r1 + r2 == j + t else w * R3 ** (r1 + r2 - j - t)

            outer = [[_strassen_lhs([[block(r1, r2, j, t) for j in range(2)] for r1 in range(2)])
                      for t in range(2)] for r2 in range(2)]
            done = [_pack(y) for r in range(7)
                    for y in _strassen_lhs([[outer[r2][t][r] for t in range(2)] for r2 in range(2)])]
            for r, y in enumerate(done):
                wd_s[r] = y
            outer = [pltpu.bitcast(z, U32) for row in outer for forms in row for z in forms]
            for i in range(RB // 16):
                yield from (z[16 * i + k:16 * i + k + 8] for z in outer for k in (0, 8))
                yield from (y[8 * i:8 * i + 8] for y in done)

        return work(), (56 + 49) * RB // 16

    def finish(b, inner):
        def work():
            for r2 in range(2):
                for s in range(2):
                    y = _strassen_out([inner[r][r2][s] for r in range(7)])
                    done = []
                    for r1 in range(2):
                        for i in range(2):
                            rows = pl.ds((2 * r1 + r2) * RB, RB)
                            tile = 2 * (1 - i) + s
                            gate = mod_s[pl.ds(5 * D + (2 * r1 + r2) * RB, RB), :]
                            z = x1_s[b, tile, rows, :] + gate * (0.125 * R3 ** -(r1 + r2 + i + s)) * y[r1][i]
                            out_v[b, rows, pl.ds(tile * T, T)] = z.astype(out_v.dtype)
                            done.append(_vregs(z))
                    yield from itertools.chain(*zip(*done))

        return work(), TPB * D // 8

    slabs = TB // (2 * MH)

    class Ffn:
        def __init__(self):
            self.order = _Order(mod_s[0:8, :])
            self.side = []
            self.due = []

        def run_under(self, work, stop, start=0):
            items, count = work
            slots = 2 * 16 * slabs
            items = itertools.chain(items, itertools.repeat(self.order.bits))
            self.side.append(_Spread(zip(*[items] * (MH // 16)), -(-count // (MH // 16)),
                                     int(stop * slots), int(start * slots)))

        def drained(self):
            return all(s.done == s.count for s in self.side)

        def lhs(self, x, due, side):
            due = [pltpu.bitcast(z, U32).reshape(-1, 16, T) for z in due]
            due = [z[:, k:k + 8].reshape(x.shape) for z in due for k in (0, 8)]
            for s in side:
                due += [jnp.concatenate(z, axis=0) for z in s.advance(1)]
            return _unpack(self.order.after(x, due))

        def next_round(self, rows):
            self.due = [(n - 1, z) for n, z in self.due]
            now = [z for n, z in self.due if n < 0 and z.shape[0] == rows]
            self.due = [(n, z) for n, z in self.due if n >= 0 or z.shape[0] != rows]
            return now

        def product(self, b, n, slab):
            def four_passes(k):
                due = self.next_round(MH)
                rows = pl.ds(slab * MH // 2, MH // 2)
                return [_dot(self.lhs(h2_s[b, 4 * k + r, rows, :], due[r::4], self.side),
                             _unpack(wgu_s[n, 4 * k + r])) for r in range(4)]

            return _gate_up_combine(four_passes)

        def gate_up(self, b, t, midway, at):
            parts = []
            for slab in range(slabs):
                g = self.product(b, 2 * t, slab)

                def silu2(i, j):
                    th = jnp.tanh(g[i][j] * (0.5 / tile_scale[2 * i + slab * MH // T]))
                    z = g[i][j] if j + t == 0 else g[i][j] * R3 ** (j + t)
                    return z + z * th

                act = [[silu2(i, j) for j in range(2)] for i in range(2)]
                self.due += [(3, z) for z in act[0] + act[1]]
                up = self.product(b, 2 * t + 1, slab)
                parts.append(_strassen_rhs([[act[1 - i][j] * up[1 - i][j] for i in range(2)] for j in range(2)]))
                self.due += [(3, z) for z in parts[-1]]
                if midway is not None and slab == at:
                    midway()
            return [jnp.concatenate(z, axis=0) for z in zip(*parts)]

        def first_half(self, b, midway=None):
            for r, z in enumerate(self.gate_up(b, 0, midway, 2)):
                act_s[b, r] = z

        def second_half(self, b, midway, at=2, last=False):
            outer = [[act_s[b, r] for r in range(7)], self.gate_up(b, 1, midway, at)]

            def down():
                rhs = [y for r in range(7)
                       for y in _strassen_rhs([[outer[t][r][:T], outer[t][r][T:]] for t in range(2)])]
                inner, m = [], {}
                for n, r in enumerate(7 * g + k for g in range(7) for k in (2, 4, 0, 3, 6, 1, 5)):
                    if n % 4 == 0:
                        due = self.next_round(RB)
                    y = acc_s[b, r] + _dot_nt(self.lhs(wd_s[r], due[n % 4::4], []), rhs[r].astype(BF16))
                    if not last:
                        acc_s[b, r] = y
                        continue
                    m[r % 7] = y
                    if n % 7 == 6:
                        inner.append(_strassen_out(m))
                        self.due += [(1, z) for z in inner[-1][0] + inner[-1][1]]
                if last:
                    self.due = [(n, z) for n, z in self.due if z.shape[0] != RB]
                    self.run_under(finish(b, inner), 0.75, 0.05)

            return down

    norm0, operands0 = project_out(0, prepare_gate_up(0))
    norm1, operands1 = project_out(1, norm0, prepare_gate_up(1))
    norm2, operands2 = project_out(2, norm1, operands0(lambda: x1_s[1, 0, 0:8]))
    norm3, operands3 = project_out(3, norm2, operands1(lambda: x1_s[2, 0, 0:8]))
    ffn = Ffn()
    fetch(0, 1).start()
    fetch(1, 1).start()
    ffn.run_under(norm3, 2, 0.5)
    ffn.run_under(operands2(lambda: x1_s[3, 0, 0:8]), 2)
    ffn.run_under(operands3(lambda: act_s[0, 0, TB // 2 - 8:]), 3, 2)
    for b in range(NB):
        ffn.first_half(b)

    def unit(u, carry):
        fetch(0, u + 1).wait()
        fetch(1, u + 1).wait()
        fetch(2, u).wait()
        ffn = Ffn()
        ffn.run_under(prepare_down(), 2.75)
        ffn.run_under(prepare_gate_up(0), NB, 2.9)
        downs = [None, None]
        for b in range(NB):
            downs.append(ffn.second_half(b, downs.pop(0)))
        assert ffn.drained()
        fetch(2, u + 1).start()
        ffn.run_under(prepare_gate_up(1), 2, 0.05)
        for b in range(NB):
            if b == 2:
                assert ffn.drained()
                fetch(0, jnp.minimum(u + 2, NU - 1)).start()
                fetch(1, jnp.minimum(u + 2, NU - 1)).start()
            ffn.first_half(b, downs.pop(0) if downs else None)
        assert ffn.drained()
        return carry

    lax.fori_loop(0, NU - 1, unit, 0)
    for n in range(3):
        fetch(n, NU - 1).wait()

    def out_copy(b):
        return pltpu.make_async_copy(out_v.at[b], out_hbm.at[:, pl.ds(b * TB, TB)], out_sem.at[b])

    ffn = Ffn()
    ffn.run_under(prepare_down(), 1.75)

    def send(b, down):
        assert ffn.drained()
        out_copy(b).start()
        down()

    down = None
    for b in range(NB):
        down = ffn.second_half(b, down, at=NB - 1 - b, last=True)
        if b > 0:
            down = functools.partial(send, b - 1, down)
    down()
    ffn.side[-1].advance(2 * ffn.side[-1].slots)
    assert ffn.drained()
    out_copy(NB - 1).start()
    for b in range(NB):
        out_copy(b).wait()


@jax.jit
def pallas_adaLN_cond__grouped_kv_mqa__swiglu_ffn__prompt_kernel(
    A_x: jax.Array,
    A_wq: jax.Array,
    A_wk: jax.Array,
    A_wv: jax.Array,
    A_wo: jax.Array,
    B_x: jax.Array,
    B_w_gate: jax.Array,
    B_w_up: jax.Array,
    B_w_down: jax.Array,
    c: jax.Array,
    w_mod: jax.Array,
):
    del B_x
    B, S, D = A_x.shape
    F = B_w_gate.shape[1]
    assert (B, S, D) == (1, T * len(VPU_GROUPS), 576) and F % FU == 0 and F > FU and A_x.dtype == BF16
    DH = D // N_HEADS
    NB, NK = S // TB, S // T
    NG = 2 * sum(VPU_GROUPS)
    vmem = pltpu.VMEM
    scratch = [
        vmem((NB, D, TB), BF16),
        vmem((D, D), BF16),
        vmem((DH, D), BF16),
        vmem((DH, D), BF16),
        vmem((D, D), BF16),
        vmem((D, FU), BF16),
        vmem((D, FU), BF16),
        vmem((D, FU), BF16),
        vmem((1, D), BF16),
        vmem((D, 6 * D), BF16),
        vmem((NB, D, TB), BF16),
        vmem((6 * D, T), F32),
        vmem(((D + 48) // 2, D), U32),
        vmem((D // 2, D), U32),
        vmem((NK, N_HEADS + 1, 24, T), F32),
        vmem((S // 16 + 3 * NK + NK * NG, 8, T), F32),
        vmem((NG, DH, 8, T), F32),
        vmem((24 + T, TB), F32),
        vmem((NK, D + 8, T), F32),
        vmem((NB, TB // T, D, T), F32),
        vmem((NB, 16, TB // 4, T), U32),
        vmem((4, 16, T // 2, T), U32),
        vmem((49, D // 8, T), U32),
        vmem((NB, 7, TB // 2, T), F32),
        vmem((NB, 49, D // 4, T), F32),
        pltpu.SMEM((1,), jnp.int32),
        pltpu.SemaphoreType.DMA((7 + NB,)),
        pltpu.SemaphoreType.DMA((3,)),
        pltpu.SemaphoreType.DMA((NB,)),
    ]
    out = pl.pallas_call(
        _kernel,
        out_shape=jax.ShapeDtypeStruct((D, S), BF16),
        in_specs=[pl.BlockSpec(memory_space=pl.ANY)] * 10,
        out_specs=pl.BlockSpec(memory_space=pl.ANY),
        scratch_shapes=scratch,
        compiler_params=pltpu.CompilerParams(vmem_limit_bytes=100 * 1024 * 1024),
        name="adaln_mqa_swiglu",
    )(A_x.reshape(S, D).T, A_wq, A_wk.T, A_wv.T, A_wo, B_w_gate, B_w_up, B_w_down.T, c, w_mod)
    return out.T.reshape(B, S, D)
```
